```python
import os as _os
_os.environ.setdefault("JAX_PLATFORMS", "cpu")
import jax
import jax.numpy as jnp

def _softmax(x, axis=-1):
    return jax.nn.softmax(x, axis=axis)
def _gelu(x):
    return jax.nn.gelu(x, approximate=True)
def _silu(x):
    return jax.nn.silu(x)
def _sigmoid(x):
    return jax.nn.sigmoid(x)
def _layernorm(x, axis=-1, eps=1e-5):
    m = jnp.mean(x, axis=axis, keepdims=True)
    v = jnp.var(x, axis=axis, keepdims=True)
    return (x - m) / jnp.sqrt(v + eps)
def _scatter_add(tgt, idx, src, axis=0):
    return tgt.at[idx].add(src)
def _segment_sum(src, seg, n):
    return jax.ops.segment_sum(src, seg, n)
class _Rng:
    def __init__(self, key):
        self._k = key
    def _next(self):
        self._k, sub = jax.random.split(self._k)
        return sub
    def normal(self, shape):
        return jax.random.normal(self._next(), shape, dtype=jnp.bfloat16)
    def randint(self, lo, hi, shape):
        return jax.random.randint(self._next(), shape, lo, hi, dtype=jnp.int32)
    def uniform(self, shape, lo=0.0, hi=1.0):
        return jax.random.uniform(self._next(), shape, jnp.bfloat16, lo, hi)
    def permutation(self, n):
        return jax.random.permutation(self._next(), n)


kernel_name = 'sequential_preLN__softmax_full_mha__geglu_ffn__prompt'

def setup_inputs():
    _rng = _Rng(jax.random.key(int.from_bytes(__import__("os").urandom(4), "little")))
    _w = (lambda a: (lambda t: t.astype(jnp.bfloat16) if jnp.issubdtype(t.dtype, jnp.floating) else t)(jnp.asarray(a)))
    def _A_setup():
        B, S, D = 1, 2048, 512
        return {
            "x": _w((lambda *s: _rng.normal(s) * 0.05)(B, S, D)),
            "wqkv": _w((lambda *s: _rng.normal(s) * 0.05)(D, 3 * D)),
            "wo": _w((lambda *s: _rng.normal(s) * 0.05)(D, D)),
        }
    _A_in = _A_setup()

    def _B_setup():
        B, S, D, F = 1, 2048, 512, 1376
        return {
            "x": _w((lambda *s: _rng.normal(s) * 0.05)(B, S, D)),
            "w_gate": _w((lambda *s: _rng.normal(s) * 0.05)(D, F)),
            "w_up": _w((lambda *s: _rng.normal(s) * 0.05)(D, F)),
            "w_down": _w((lambda *s: _rng.normal(s) * 0.05)(F, D)),
        }
    _B_in = _B_setup()

    return {
        "A_x": _A_in["x"],
        "A_wqkv": _A_in["wqkv"],
        "A_wo": _A_in["wo"],
        "B_x": _B_in["x"],
        "B_w_gate": _B_in["w_gate"],
        "B_w_up": _B_in["w_up"],
        "B_w_down": _B_in["w_down"],
    }

def reference(A_x, A_wqkv, A_wo, B_x, B_w_gate, B_w_up, B_w_down):
    def _A_ref(x, wqkv, wo):
        B, S, D = x.shape
        H = 32; Dh = D // H
        qkv = (lambda x, *d: x.transpose(*d))((x @ wqkv).reshape(B, S, 3, H, Dh), 2, 0, 3, 1, 4)
        q, k, v = qkv[0], qkv[1], qkv[2]
        scale = Dh ** -0.5
        scores = jnp.einsum("bhqd,bhkd->bhqk", q, k) * scale
        p = _softmax(scores, axis=-1)
        o = jnp.einsum("bhqk,bhkd->bhqd", p, v)
        return (lambda x, *d: x.transpose(*d))(o, 0, 2, 1, 3).reshape(B, S, D) @ wo

    def _B_ref(x, w_gate, w_up, w_down):
        return (_gelu(x @ w_gate) * (x @ w_up)) @ w_down

    x = A_x
    h = x + _A_ref(_layernorm(x, axis=-1), A_wqkv, A_wo)
    h2 = h + _B_ref(_layernorm(h, axis=-1), B_w_gate, B_w_up, B_w_down)
    return h2
```

```python
import functools
import math
import os

import jax
import jax.numpy as jnp
from jax import lax
import jax.experimental.pallas as pl
import jax.experimental.pallas.tpu as pltpu

_BF = jnp.bfloat16
_F32 = jnp.float32
_U32 = jnp.uint32

_H = 32
_DH = 16
_EPS = 1e-5
_TQ = 512
_TK = 256
_CFG = dict(R=32, RB=16, CB=256, KP=32, R1=512, R3=256, NSUB=2, P1LOOP=0)
for _kv in os.environ.get("KCFG", "").split(","):
    if _kv:
        _k, _v = _kv.split("=")
        _CFG[_k] = int(_v)
_RV = _CFG["R"]
_RB = _CFG["RB"]
_CB = _CFG["CB"]
_KP = _CFG["KP"]
_R1 = _CFG["R1"]
_R3 = _CFG["R3"]
_NSUB = _CFG["NSUB"]
_NZ = 256
_L_LO = 2.0 ** -40
_L_HI = 2.0 ** 60
_V_HI = 2.0 ** 50


def _layernorm(x):
    m = jnp.mean(x, axis=-1, keepdims=True)
    xc = x - m
    v = jnp.mean(xc * xc, axis=-1, keepdims=True)
    return xc * lax.rsqrt(v + _EPS)


def _gelu_tanh(x):
    c = math.sqrt(2.0 / math.pi)
    return 0.5 * x * (1.0 + jnp.tanh(c * (x + 0.044715 * (x * x * x))))


def _as_bf16(x):
    return pltpu.bitcast(x, _BF)


def _pack_rows(x):
    cols = [pltpu.bitcast(x[:, c:c + 128].astype(_BF), _U32) for c in range(0, x.shape[1], 128)]
    return cols[0] if len(cols) == 1 else jnp.concatenate(cols, axis=1)


def _pack_interleaved(x):
    n = x.shape[0] // 16
    x4 = x.reshape(n, 2, 8, x.shape[1])
    return pltpu.pack_elementwise([x4[:, 0], x4[:, 1]], packed_dtype=_BF).reshape(n * 8, x.shape[1])


def _dot(a, b):
    return jnp.dot(a, b, preferred_element_type=_F32)


def _dot_nt(a, b):
    return lax.dot_general(a, b, (((1,), (1,)), ((), ())), preferred_element_type=_F32)


def _dot_tn(a, b):
    return lax.dot_general(a, b, (((0,), (0,)), ((), ())), preferred_element_type=_F32)


def _kernel(x_hbm, wqkv_hbm, wo_hbm, wgt_hbm, wut_hbm, wd_hbm, out_hbm,
            x_s, wqkv_s, wo_s, wgt_s, wut_s, wd_s, out_s, wqvt_s,
            k_s, kf_s, vt_s, qm_s, qf_s, acc_s, l_s, z_s, b00, b01, b10, b11, sems,
            *, S, D):
    nq = S // _TQ
    nc = S // _TK
    ng = D // 128
    nb1 = S // _R1
    koff = _RV * nc
    prows = 4 * (_TK // 2)
    bufs = ((b00, b01), (b10, b11))
    qscale = (_DH ** -0.5) * math.log2(math.e)

    def x_copy(b):
        rows = pl.ds(b * _R1, _R1)
        return pltpu.make_async_copy(x_hbm.at[rows, :], x_s.at[rows, :], sems.at[b])

    def w_copy(c):
        cols = pl.ds(c * D, D)
        return pltpu.make_async_copy(wqkv_hbm.at[:, cols], wqkv_s.at[:, cols], sems.at[nb1 + c])

    late = [pltpu.make_async_copy(src, dst, sems.at[nb1 + 3 + i])
            for i, (src, dst) in enumerate(((wo_hbm, wo_s), (wgt_hbm, wgt_s),
                                            (wut_hbm, wut_s), (wd_hbm, wd_s)))]
    osem0 = nb1 + 7

    x_copy(0).start()
    w_copy(1).start()
    w_copy(0).start()
    w_copy(2).start()
    for b in range(1, nb1):
        x_copy(b).start()
    for cp in late:
        cp.start()

    for i in range(_NZ):
        z_s[i] = 0
    for h in range(_H):
        j = h % 8
        if j > 0:
            qm_s[h, 0:j * 8, :] = jnp.zeros((j * 8, S), _U32)
        if j < 7:
            qm_s[h, (j + 1) * 8:64, :] = jnp.zeros(((7 - j) * 8, S), _U32)

    vmax = None
    for rb in range(nb1):
        rows = slice(rb * _R1, (rb + 1) * _R1)
        x_copy(rb).wait()
        xn32 = _layernorm(x_s[rows, :].astype(_F32))
        xn = xn32.astype(_BF)
        xi = _as_bf16(_pack_interleaved(xn32))
        if rb == 0:
            w_copy(1).wait()
        k = _dot(xn, wqkv_s[:, D:2 * D])
        for g in range(ng):
            k_s[g, rb * _R1 // 2:(rb + 1) * _R1 // 2, :] = _pack_rows(k[:, g * 128:(g + 1) * 128])
            for kc in range(_R1 // _TK):
                if _RV:
                    c = rb * (_R1 // _TK) + kc
                    kf_s[g, c * _RV:(c + 1) * _RV, :] = k[(kc + 1) * _TK - _RV:(kc + 1) * _TK,
                                                          g * 128:(g + 1) * 128]
        if rb == 0:
            w_copy(0).wait()
            wqvt_s[0:D, :] = wqkv_s[:, 0:D].T
            w_copy(2).wait()
            wqvt_s[D:2 * D, :] = wqkv_s[:, 2 * D:3 * D].T
        qt = _dot_nt(wqvt_s[0:D, :], xn) * qscale
        qp = _pack_rows(qt)
        for h in range(_H):
            j = h % 8
            qm_s[h, j * 8:(j + 1) * 8, rows] = qp[h * 8:(h + 1) * 8]
            if _RV:
                qf_s[h, :, rows] = qt[h * _DH:(h + 1) * _DH]
        vt = _dot_nt(wqvt_s[D:2 * D, :], xi)
        vp = _pack_rows(vt)
        for h in range(_H):
            vt_s[h, :, rows] = vp[h * 8:(h + 1) * 8]
        vm = jnp.max(jnp.abs(vt).reshape(D // 8, 8, _R1), axis=0)
        vmax = vm if vmax is None else jnp.maximum(vmax, vm)

    def kb_piece(h, u, d, r0, nr):
        idx = jnp.full((nr, 128), (h % 8) * _DH + d, jnp.int32)
        kbv = jnp.take_along_axis(kf_s[h // 8, r0:r0 + nr, :], idx, axis=1)
        row = prows + (d // 2) * koff + r0
        bufs[u][d % 2][0, row:row + nr, :] = pltpu.bitcast(kbv, _U32)

    if _RV:
        for d in range(_DH):
            kb_piece(0, 0, d, 0, koff)

    def pair_body(hh, carry):
        lmin, lmax = carry
        items = [(u, qb, kc) for u in range(2) for qb in range(nq) for kc in range(nc)]
        nper = nq * nc
        nm = _TK - _RV
        cnt = [0]
        z1 = z_s[_NZ - 2]
        z2 = z_s[_NZ - 1]

        def vtask(buf, u, qb, kc, r0, c0, lsum):
            z = z_s[cnt[0] % (_NZ - 2)]
            cnt[0] += 1
            qv = qf_s.at[hh * 2 + u + z]
            accs = [None] * (_CB // 128)
            for d in range(_DH):
                row = prows + (d // 2) * koff + kc * _RV + r0
                kb = pltpu.bitcast(bufs[u][d % 2][z, row:row + _RB, :], _F32)
                for cc in range(_CB // 128):
                    col = qb * _TQ + c0 + cc * 128
                    t = kb * qv[d:d + 1, col:col + 128]
                    accs[cc] = t if accs[cc] is None else accs[cc] + t
            r = nm + r0
            for cc in range(_CB // 128):
                p = jnp.exp2(accs[cc])
                ps = jnp.sum(p.reshape(_RB // 8, 8, 128), axis=0)
                ct = c0 // 128 + cc
                lsum[ct] = ps if lsum.get(ct) is None else lsum[ct] + ps
                base = ct * (_TK // 2)
                buf[z2, base + r // 2:base + (r + _RB) // 2, :] = _pack_interleaved(p)

        def qk(u, qb, kc):
            h = hh * 2 + u
            kk = _as_bf16(k_s[h // 8, kc * _TK // 2:(kc * _TK + nm) // 2, :])
            return _dot(kk, _as_bf16(qm_s[h, :, qb * _TQ:(qb + 1) * _TQ]))

        kbl = [[(d, r0) for d in range(par, _DH, 2) for r0 in range(0, koff, _KP)]
               for par in range(2)]

        def softmax_item(i, s, st):
            u, qb, kc = items[i]
            buf = bufs[1 - u][i % 2]
            tl = [(r0, c0) for r0 in range(0, _RV, _RB) for c0 in range(0, _TQ, _CB)]
            ii = i % nper
            usable = [t for t in range(2, nper - 2) if t % 2 == i % 2]
            kl = []
            if ii in usable:
                lst = kbl[i % 2]
                a = usable.index(ii)
                kl = lst[len(lst) * a // len(usable):len(lst) * (a + 1) // len(usable)]
            hn = jnp.minimum(hh * 2 + u + 1, _H - 1)
            npc = nm // 16
            dn = 0
            dk = 0
            for pi in range(npc):
                p = jnp.exp2(s[pi * 16:(pi + 1) * 16])
                ps = p[0:8] + p[8:16]
                st["l8"] = ps if st.get("l8") is None else st["l8"] + ps
                pp = _pack_interleaved(p)
                for ct in range(_TQ // 128):
                    base = ct * (_TK // 2) + pi * 8
                    buf[z1, base:base + 8, :] = pp[:, ct * 128:(ct + 1) * 128]
                while dn < (len(tl) * (pi + 1)) // npc:
                    vtask(buf, u, qb, kc, *tl[dn], st["ls"])
                    dn += 1
                while dk < (len(kl) * (pi + 1)) // npc:
                    kb_piece(hn, 1 - u, kl[dk][0], kl[dk][1], min(_KP, koff - kl[dk][1]))
                    dk += 1

        n = len(items)
        sts = {}
        for i in range(-1, n):
            if i + 1 < n:
                s = qk(*items[i + 1])
            if i >= 0:
                u, qb, kc = items[i]
                h = hh * 2 + u
                buf = bufs[1 - u][i % 2]
                pm = jnp.concatenate(
                    [buf[0, ct * (_TK // 2):(ct + 1) * (_TK // 2), :] for ct in range(_TQ // 128)],
                    axis=1)
                pv = _dot(_as_bf16(vt_s[h, :, kc * _TK:(kc + 1) * _TK]), _as_bf16(pm))
                acc = pv if kc == 0 else pv + acc
                if kc == nc - 1:
                    st = sts.pop((u, qb))
                    l8 = st["l8"]
                    if _RV:
                        l8 = l8 + jnp.concatenate(
                            [st["ls"][ct] for ct in range(_TQ // 128)], axis=1)
                    acc_s[h, :, qb * _TQ:(qb + 1) * _TQ] = acc
                    l_s[h, :, qb * _TQ:(qb + 1) * _TQ] = l8
                    lmin = jnp.minimum(lmin, l8)
                    lmax = jnp.maximum(lmax, l8)
            if i + 1 < n:
                u, qb, kc = items[i + 1]
                softmax_item(i + 1, s, sts.setdefault((u, qb), dict(ls={})))
        return lmin, lmax

    ones = jnp.ones((8, _TQ), _F32)
    lmin, lmax = lax.fori_loop(0, _H // 2, pair_body, (ones, ones))
    ok = jnp.logical_and(jnp.logical_and(lmin >= _L_LO, lmax <= _L_HI),
                         vmax <= _V_HI)
    nbad = jnp.sum(jnp.where(ok, 0.0, 1.0))

    @pl.when(nbad > 0.0)
    def _():
        def exact(t, c):
            h = t // nq
            cols = pl.ds(pl.multiple_of((t % nq) * _TQ, _TQ), _TQ)
            s = _dot(_as_bf16(k_s[h // 8]), _as_bf16(qm_s[h, :, cols]))
            p = jnp.exp2(s - jnp.max(s, axis=0, keepdims=True))
            l8 = jnp.sum(p.reshape(S // 8, 8, _TQ), axis=0)
            p = p * (1.0 / jnp.sum(l8, axis=0, keepdims=True))
            acc_s[h, :, cols] = _dot(_as_bf16(vt_s[h]), _as_bf16(_pack_interleaved(p)))
            l_s[h, :, cols] = jnp.full((8, _TQ), 0.125, _F32)
            return c
        lax.fori_loop(0, _H * nq, exact, 0)

    for cp in late:
        cp.wait()

    rblk = _R3 * _NSUB

    def out_copy(t):
        rows = pl.ds(pl.multiple_of(t * rblk, rblk), rblk)
        return pltpu.make_async_copy(out_s.at[rows, :], out_hbm.at[rows, :], sems.at[osem0 + t])

    def ffn_body(t, c):
        subs = [pl.ds(pl.multiple_of(t * rblk + i * _R3, _R3), _R3) for i in range(_NSUB)]
        h1 = []
        for rows in subs:
            l = jnp.sum(l_s[:, :, rows], axis=1, keepdims=True)
            ot = (acc_s[:, :, rows] * (1.0 / l)).reshape(D, _R3).astype(_BF)
            h1.append(x_s[rows, :].astype(_F32) + _dot_tn(ot, wo_s[...]))
        act = []
        for i in range(_NSUB):
            hn = _layernorm(h1[i]).astype(_BF)
            gate = _dot_nt(hn, wgt_s[...])
            up = _dot_nt(hn, wut_s[...])
            act.append((_gelu_tanh(gate) * up).astype(_BF))
        for i, rows in enumerate(subs):
            out_s[rows, :] = (_dot(act[i], wd_s[...]) + h1[i]).astype(_BF)
        out_copy(t).start()
        return c

    lax.fori_loop(0, S // rblk, ffn_body, 0)
    for t in range(S // rblk):
        out_copy(t).wait()


@jax.jit
def pallas_sequential_preLN__softmax_full_mha__geglu_ffn__prompt_kernel(
    A_x, A_wqkv, A_wo, B_x, B_w_gate, B_w_up, B_w_down,
):
    B, S, D = A_x.shape
    F = B_w_gate.shape[1]
    koff = max(_RV * (S // _TK), 8)
    brows = 4 * (_TK // 2) + (_DH // 2) * koff
    nsem = S // _R1 + 7 + S // (_R3 * _NSUB)
    hbm = pl.BlockSpec(memory_space=pl.ANY)
    out = pl.pallas_call(
        functools.partial(_kernel, S=S, D=D),
        in_specs=[hbm] * 6,
        out_specs=hbm,
        out_shape=jax.ShapeDtypeStruct((S, D), A_x.dtype),
        scratch_shapes=[
            pltpu.VMEM((S, D), _BF),
            pltpu.VMEM((D, 3 * D), _BF),
            pltpu.VMEM((D, D), _BF),
            pltpu.VMEM((F, D), _BF),
            pltpu.VMEM((F, D), _BF),
            pltpu.VMEM((F, D), _BF),
            pltpu.VMEM((S, D), _BF),
            pltpu.VMEM((2 * D, D), _BF),
            pltpu.VMEM((D // 128, S // 2, 128), _U32),
            pltpu.VMEM((D // 128, koff, 128), _F32),
            pltpu.VMEM((_H, _DH // 2, S), _U32),
            pltpu.VMEM((_H, 64, S), _U32),
            pltpu.VMEM((_H, _DH, S), _F32),
            pltpu.VMEM((_H, _DH, S), _F32),
            pltpu.VMEM((_H, 8, S), _F32),
            pltpu.SMEM((_NZ,), jnp.int32),
            pltpu.VMEM((2, brows, 128), _U32),
            pltpu.VMEM((2, brows, 128), _U32),
            pltpu.VMEM((2, brows, 128), _U32),
            pltpu.VMEM((2, brows, 128), _U32),
            pltpu.SemaphoreType.DMA((nsem,)),
        ],
        compiler_params=pltpu.CompilerParams(
            vmem_limit_bytes=110 * 1024 * 1024,
        ),
        name="fused_block",
    )(A_x.reshape(S, D), A_wqkv, A_wo, B_w_gate.T, B_w_up.T, B_w_down)
    return out.reshape(B, S, D)
```

```python
import functools
import math

import jax
import jax.numpy as jnp
from jax import lax
import jax.experimental.pallas as pl
import jax.experimental.pallas.tpu as pltpu

_BF = jnp.bfloat16
_F32 = jnp.float32

_H = 32
_DH = 16
_EPS = 1e-5
_TQ = 512
_TK = 256
_RB = 16
_CB = 256
_R1 = 512
_R3 = 256
_NSUB = 2
_NZ = 256

_L_LO = 2.0 ** -40
_L_HI = 2.0 ** 60
_V_HI = 2.0 ** 50

_VPU_ROWS = "22222222223223222323232323232323"
_EXTRA0 = 16
_KP = 32
_RP = 32
_PV_SLOTS = 2.0
_P_LOAD0 = 5
_K_PRE0 = 3


def _layernorm(x):
    m = jnp.mean(x, axis=-1, keepdims=True)
    xc = x - m
    v = jnp.mean(xc * xc, axis=-1, keepdims=True)
    return xc * lax.rsqrt(v + _EPS)


def _gelu_tanh(x):
    c = math.sqrt(2.0 / math.pi)
    return 0.5 * x * (1.0 + jnp.tanh(c * (x + 0.044715 * (x * x * x))))


def _recip(x):
    r = pl.reciprocal(x, approx=True)
    return r * (2.0 - x * r)


def _pack(x):
    return pltpu.bitcast(x.astype(_BF), _F32)


def _unpack(x):
    return pltpu.bitcast(x, _BF)


def _dot(a, b):
    return lax.dot_general(a, b, (((1,), (0,)), ((), ())), preferred_element_type=_F32)


def _dot_nt(a, b):
    return lax.dot_general(a, b, (((1,), (1,)), ((), ())), preferred_element_type=_F32)


def _dot_tn(a, b):
    return lax.dot_general(a, b, (((0,), (0,)), ((), ())), preferred_element_type=_F32)


def _vpu_rows(S):
    nc = S // _TK
    nq = S // _TQ
    rl = [[16 * int(_VPU_ROWS[qb * nc + kc]) for kc in range(nc)] for qb in range(nq)]
    rmax = [max(rl[qb][kc] for qb in range(nq)) for kc in range(nc)]
    rmin = [min(rl[qb][kc] for qb in range(nq)) for kc in range(nc)]
    rmax[0] = max(rmax[0], rl[0][0] + _EXTRA0)
    return rl, rmax, rmin


def _make_plan(S, first):
    nc = S // _TK
    nper = (S // _TQ) * nc
    rl, rmax, rmin = _vpu_rows(S)
    extra = _EXTRA0 if first else 0
    rv = [rl[i // nc][i % nc] for i in range(nper)]
    rv[0] += extra
    npcs = [(_TK - r) // 16 for r in rv]
    starts = [sum(n + _PV_SLOTS for n in npcs[:i]) + _PV_SLOTS for i in range(nper)]
    ends = [starts[i] + npcs[i] for i in range(nper)]

    def place(pos):
        i = min(t for t in range(nper) if pos <= ends[t] + 1e-6)
        return i, max(0, int(math.floor(pos - starts[i] + 1e-6)))

    tasks = [(i, r0, c0) for i in range(nper)
             for r0 in range(0, rv[i], _RB) for c0 in range(0, _TQ, _CB)]
    nx = (extra // _RB) * (_TQ // _CB)
    sched = {}
    for j, (i, r0, c0) in enumerate(tasks):
        q0 = (i // nc) * nc
        peers = [t for t in range(nx, len(tasks)) if tasks[t][0] // nc == i // nc]
        beg = starts[q0] - _PV_SLOTS
        pos = beg + (j + 1 - peers[0]) * (ends[q0 + nc - 1] - beg) / len(peers)
        pos = min(max(pos, starts[i - 1] if i > 0 else 0.0), ends[i])
        sched.setdefault(place(pos), []).append(("score", i, r0, c0))
    bcast = [("bcast", d, r0) for d in range(_DH) for r0 in range(0, sum(rmax), _KP)]
    roll = [("roll", kc, r0) for kc in range(nc) for r0 in range(0, (_TK - rmin[kc]) // 2, _RP)]
    for lst in (bcast, roll):
        for j, e in enumerate(lst):
            pos = starts[1] + (j + 0.5) * (ends[nper - 2] - starts[1]) / len(lst)
            sched.setdefault(place(pos), []).append(e)
    return rv, npcs, sched


def _kernel(x_hbm, wqkv_hbm, wo_hbm, wgt_hbm, wut_hbm, wd_hbm, out_hbm,
            x_s, wqkv_s, wo_s, wgt_s, wut_s, wd_s, out_s, wqvt_s, o_s,
            k_s, kf_s, vt_s, qt_s, qf_s, acc_s, l_s, z_s, b0, b1, sems,
            *, S, D):
    nq = S // _TQ
    nc = S // _TK
    ng = D // 128
    nb1 = S // _R1
    nper = nq * nc
    _, rmax, rmin = _vpu_rows(S)
    roff = [sum(rmax[:i]) for i in range(nc)]
    koff = sum(rmax)
    half = _TK // 2
    lrow = 4 * half
    rrow = lrow + 24
    krow = rrow + S // 8
    bufs = (b0, b1)
    qscale = (_DH ** -0.5) * math.log2(math.e)

    def x_copy(b, sem):
        rows = pl.ds(b * _R1, _R1)
        return pltpu.make_async_copy(x_hbm.at[rows, :], x_s.at[rows, :], sems.at[sem])

    def w_copy(c, sem):
        cols = pl.ds(c * D, D)
        return pltpu.make_async_copy(wqkv_hbm.at[:, cols], wqkv_s.at[:, cols], sems.at[sem])

    def group2():
        return [x_copy(1, 2), w_copy(0, 2)]

    def group3():
        return [x_copy(b, 3) for b in range(2, nb1)] + [w_copy(2, 3)]

    def late_copies():
        return [pltpu.make_async_copy(src, dst, sems.at[4])
                for src, dst in ((wo_hbm, wo_s), (wgt_hbm, wgt_s), (wut_hbm, wut_s), (wd_hbm, wd_s))]

    def ln_block(rb):
        return _layernorm(x_s[rb * _R1:(rb + 1) * _R1, :].astype(_F32)).astype(_BF)

    def k_block(rb, xn, split=1):
        nr = _R1 // split
        for r in range(0, _R1, nr):
            r0 = rb * _R1 + r
            k = _dot(xn[r:r + nr], wqkv_s[:, D:2 * D])
            for g in range(ng):
                lanes = slice(g * 128, (g + 1) * 128)
                k_s[g, r0 // 2:(r0 + nr) // 2, :] = _pack(k[:, lanes])
                for c in range(nc):
                    end = (c + 1) * _TK
                    if r0 < end <= r0 + nr:
                        kf_s[g, roff[c]:roff[c] + rmax[c], :] = k[end - r0 - rmax[c]:end - r0, lanes]

    def q_block(rb, xn):
        rows = slice(rb * _R1, (rb + 1) * _R1)
        qt = _dot_nt(wqvt_s[0:D, :], xn) * qscale
        for h in range(_H):
            qh = qt[h * _DH:(h + 1) * _DH]
            qt_s.at[h][:, rows] = _pack(qh)
            qf_s[h, :, rows] = qh

    def v_block(rb, xn):
        rows = slice(rb * _R1, (rb + 1) * _R1)
        vt = _dot_nt(wqvt_s[D:2 * D, :], xn)
        for h in range(_H):
            vt_s.at[h][:, rows] = _pack(vt[h * _DH:(h + 1) * _DH])
        return jnp.max(jnp.abs(vt).reshape(D // 8, 8, _R1), axis=0)

    def bcast_piece(h, u, d, r0, nr):
        idx = jnp.full((nr, 128), (h % 8) * _DH + d, jnp.int32)
        row = krow + (d // 4) * koff + r0
        col = (d % 4) * 128
        bufs[u][0, row:row + nr, col:col + 128] = jnp.take_along_axis(
            kf_s[h // 8, r0:r0 + nr, :], idx, axis=1)

    def k_slot(kc, r0):
        return rrow + (kc // 4) * half + r0, (kc % 4) * 128

    def rolled_keys(h, rows):
        return pltpu.roll(k_s[h // 8, rows, :], (128 - (h % 8) * _DH) % 128, 1)

    def roll_piece(h, u, kc, r0, nr):
        row, col = k_slot(kc, r0)
        bufs[u][0, row:row + nr, col:col + 128] = rolled_keys(
            h, slice(kc * half + r0, kc * half + r0 + nr))

    x_copy(0, 0).start()
    w_copy(1, 1).start()
    for i in range(_NZ):
        z_s[i] = 0
    b0[0, 2 * half:4 * half, :] = jnp.zeros((2 * half, _TQ), _F32)
    x_copy(0, 0).wait()
    for cp in group2():
        cp.start()
    xns = [ln_block(0)]
    w_copy(1, 1).wait()
    k_block(0, xns[0])
    for cp in group2():
        cp.wait()
    for cp in group3():
        cp.start()
    xns.append(ln_block(1))
    k_block(1, xns[1], 4)
    wqvt_s[0:D, :] = wqkv_s[:, 0:D].T
    q_block(0, xns[0])
    for cp in group3():
        cp.wait()
    for cp in late_copies():
        cp.start()
    q_block(1, xns[1])
    for rb in range(2, nb1):
        xns.append(ln_block(rb))
        k_block(rb, xns[rb])
    wqvt_s[D:2 * D, :] = wqkv_s[:, 2 * D:3 * D].T
    for d in range(_DH):
        bcast_piece(0, 0, d, 0, koff)
    for kc in range(nc):
        roll_piece(0, 0, kc, 0, half)
    vmax = None
    for rb, xn in enumerate(xns):
        if rb > 1:
            q_block(rb, xn)
        vm = v_block(rb, xn)
        vmax = vm if vmax is None else jnp.maximum(vmax, vm)
    for cp in late_copies():
        cp.wait()

    def p_group(buf, slot, g):
        cols = slice((g // 8) * 256, (g // 8 + 1) * 256)
        sub = 7 - g % 8
        return [buf[0, slot * half + (kt * 8 + sub) * 8:slot * half + (kt * 8 + sub + 1) * 8, cols]
                for kt in range(2)]

    def pv_dot(h, kc, groups):
        sets = []
        for st in range(2):
            rows = [groups[st * 8 + 7 - sub][kt] for kt in range(2) for sub in range(8)]
            sets.append(jnp.concatenate(rows, axis=0))
        pm = jnp.concatenate(sets, axis=1)
        return _dot(_unpack(vt_s[h, :, kc * _TK:(kc + 1) * _TK]), _unpack(pm))

    plans = [_make_plan(S, u == 0) for u in range(2)]

    def pair_body(hh, acc):
        cnt = [0]
        z1 = z_s[_NZ - 2]
        z2 = z_s[_NZ - 1]

        def score_task(u, i, r0, c0, lsum, tail):
            qb, kc = divmod(i, nc)
            rv = plans[u][0][i]
            dst = bufs[1 - u].at[z2]
            z = z_s[cnt[0] % (_NZ - 2)]
            cnt[0] += 1
            qv = qf_s.at[hh * 2 + u + z]
            kv = bufs[u].at[z]
            accs = [None] * (_CB // 128)
            for d in range(_DH):
                row = krow + (d // 4) * koff + roff[kc] + rmax[kc] - rv + r0
                kb = kv[row:row + _RB, (d % 4) * 128:(d % 4 + 1) * 128]
                for cc in range(_CB // 128):
                    col = qb * _TQ + c0 + cc * 128
                    t = kb * qv[d:d + 1, col:col + 128]
                    accs[cc] = t if accs[cc] is None else accs[cc] + t
            r = (i % 4) * _TK + _TK - rv + r0
            vrow = lrow + (qb % 2) * 8
            for cc in range(_CB // 128):
                p = jnp.exp2(accs[cc])
                ps = p[0:8] + p[8:16]
                ct = c0 // 128 + cc
                lanes = slice(ct * 128, (ct + 1) * 128)
                dst[r // 2:(r + _RB) // 2, lanes] = _pack(p)
                if ct in lsum:
                    ps = lsum[ct] + ps
                elif ct in tail:
                    ps = ps + jnp.minimum(tail[ct], 0.0)
                lsum[ct] = ps
                tail[ct] = ps
                dst[vrow:vrow + 8, lanes] = ps

        loaded = {}
        kpre = []
        for u in range(2):
            h = hh * 2 + u
            hn = jnp.minimum(h + 1, _H - 1)
            buf = bufs[1 - u]
            rvs, npcs, sched = plans[u]
            tail = {}
            lsums = [dict() for _ in range(nq)]

            def side_work(i, pi):
                for e in sched.get((i, pi), []):
                    if e[0] == "score":
                        score_task(u, e[1], e[2], e[3], lsums[e[1] // nc], tail)
                    elif e[0] == "bcast":
                        bcast_piece(hn, 1 - u, e[1], e[2], min(_KP, koff - e[2]))
                    else:
                        roll_piece(hn, 1 - u, e[1], e[2],
                                   min(_RP, (_TK - rmin[e[1]]) // 2 - e[2]))

            for i in range(nper):
                qb, kc = divmod(i, nc)
                cols = slice(qb * _TQ, (qb + 1) * _TQ)
                row, col = k_slot(kc, 0)
                kparts = kpre if (u == 1 and i == 0) else []
                kparts.append(bufs[u][0, row + 8 * len(kparts):row + (_TK - rvs[i]) // 2,
                                      col:col + 128])
                kk = _unpack(jnp.concatenate(kparts, axis=0) if len(kparts) > 1 else kparts[0])
                s = _dot(kk[:, 0:_DH], _unpack(qt_s[h, :, cols]))

                i2 = (i - 2) % nper
                pqb, pkc = divmod(i2, nc)
                ph = h if i >= 2 else jnp.maximum(h - 1, 0)
                groups = loaded.pop((u, i2) if i >= 2 else (u - 1, i2), None)
                if groups is None:
                    groups = [p_group(bufs[u], i2 % 4, g) for g in range(16)]
                pv = pv_dot(ph, pkc, groups)
                acc = pv if pkc == 0 else pv + acc
                if pkc == nc - 1:
                    acc_s[ph, :, pqb * _TQ:(pqb + 1) * _TQ] = acc

                reload = i >= 1 and not (u == 1 and i == nper - 1)
                groups = []
                side_work(i, 0)
                for pi in range(npcs[i]):
                    p = jnp.exp2(s[pi * 16:(pi + 1) * 16])
                    ps = p[0:8] + p[8:16]
                    l8 = ps if (kc == 0 and pi == 0) else l8 + ps
                    row = (i % 4) * half + pi * 8
                    buf.at[z1][row:row + 8, :] = _pack(p)
                    side_work(i, pi + 1)
                    if u == 0 and i == nper - 1 and _K_PRE0 <= pi < npcs[i] - 1:
                        krow0, kcol0 = k_slot(0, 8 * len(kpre))
                        kpre.append(buf[0, krow0:krow0 + 8, kcol0:kcol0 + 128])
                    if reload:
                        want = max(0, (16 * (pi + 1 - _P_LOAD0)) // (npcs[i] - _P_LOAD0))
                        while len(groups) < want:
                            groups.append(p_group(buf, (i - 1) % 4, len(groups)))
                if reload:
                    loaded[(u, i - 1)] = groups
                if kc == nc - 1:
                    buf.at[z1][lrow + 16:lrow + 24, :] = l8
                    vrow = lrow + (qb % 2) * 8
                    l_s[h, :, cols] = buf[0, lrow + 16:lrow + 24, :] + buf[0, vrow:vrow + 8, :]
        return acc

    acc = lax.fori_loop(0, _H // 2, pair_body, jnp.zeros((_DH, _TQ), _F32))
    for j in (2, 1):
        acc = pv_dot(_H - 1, nc - j, [p_group(b0, (nper - j) % 4, g) for g in range(16)]) + acc
    acc_s[_H - 1, :, S - _TQ:S] = acc

    def max_shifted_attention():
        nt = S // 128

        def tile(t, c):
            h = t // nt
            cols = pl.ds(pl.multiple_of((t % nt) * 128, 128), 128)
            kk = _unpack(rolled_keys(h, slice(None)))
            s = _dot(kk[:, 0:_DH], _unpack(qt_s[h, :, cols]))
            p = jnp.exp2(s - jnp.max(s, axis=0, keepdims=True))
            p = p * (1.0 / jnp.sum(p, axis=0, keepdims=True))
            acc_s[h, :, cols] = _dot(_unpack(vt_s[h]), p.astype(_BF))
            l_s[h, :, cols] = jnp.full((8, 128), 0.125, _F32)
            return c
        lax.fori_loop(0, _H * nt, tile, 0)

    rblk = _R3 * _NSUB
    nblk = S // rblk

    def attn_rows(rows):
        l = jnp.sum(l_s[:, :, rows], axis=1, keepdims=True)
        ot = (acc_s[:, :, rows] * _recip(l)).reshape(D, _R3).astype(_BF)
        ok = jnp.logical_and(l >= _L_LO, l <= _L_HI)
        return ot.T, jnp.sum(jnp.where(ok, 0.0, 1.0), axis=0)

    def ffn_body(t, bad):
        subs = [pl.ds(pl.multiple_of(t * rblk + i * _R3, _R3), _R3) for i in range(_NSUB)]
        h1 = []
        for i, rows in enumerate(subs):
            if i == 0:
                o = o_s[...]
            else:
                o, b = attn_rows(rows)
                bad = bad + b
            h1.append(_dot(o, wo_s[...]) + x_s[rows, :].astype(_F32))
        act = []
        for i in range(_NSUB):
            hn = _layernorm(h1[i]).astype(_BF)
            gate = _dot_nt(wgt_s[...], hn)
            up = _dot_nt(wut_s[...], hn)
            act.append((_gelu_tanh(gate) * up).astype(_BF))
        nxt = jnp.minimum(t + 1, nblk - 1) * rblk
        o_s[...], b = attn_rows(pl.ds(pl.multiple_of(nxt, _R3), _R3))
        bad = bad + b
        for i, rows in enumerate(subs):
            out_s[rows, :] = (_dot_tn(act[i], wd_s[...]) + h1[i]).astype(_BF)
            pltpu.make_async_copy(out_s.at[rows, :], out_hbm.at[rows, :], sems.at[5]).start()
        return bad

    o_s[...], bad0 = attn_rows(pl.ds(0, _R3))
    vmax = jnp.max(vmax, axis=0, keepdims=True)
    for c in range(0, _R1, _R3):
        bad0 = bad0 + jnp.where(vmax[:, c:c + _R3] <= _V_HI, 0.0, 1.0)

    def one_pass(state):
        p, _ = state
        bad = lax.fori_loop(0, nblk, ffn_body, bad0)
        redo = jnp.logical_and(p == 0, jnp.sum(bad) > 0.0)

        @pl.when(redo)
        def _():
            max_shifted_attention()
            o_s[...] = attn_rows(pl.ds(0, _R3))[0]

        pltpu.make_async_copy(out_s, out_hbm, sems.at[5]).wait()
        return p + 1, redo.astype(jnp.int32)

    lax.while_loop(lambda st: st[1] > 0, one_pass, (jnp.int32(0), jnp.int32(1)))


@jax.jit
def pallas_sequential_preLN__softmax_full_mha__geglu_ffn__prompt_kernel(
    A_x: jax.Array,
    A_wqkv: jax.Array,
    A_wo: jax.Array,
    B_x: jax.Array,
    B_w_gate: jax.Array,
    B_w_up: jax.Array,
    B_w_down: jax.Array,
):
    B, S, D = A_x.shape
    F = B_w_gate.shape[1]
    assert B == 1 and D == _H * _DH and len(_VPU_ROWS) == (S // _TQ) * (S // _TK)
    koff = sum(_vpu_rows(S)[1])
    brows = 2 * _TK + 24 + S // 8 + 4 * koff
    hbm = pl.BlockSpec(memory_space=pl.ANY)
    out = pl.pallas_call(
        functools.partial(_kernel, S=S, D=D),
        in_specs=[hbm] * 6,
        out_specs=hbm,
        out_shape=jax.ShapeDtypeStruct((S, D), A_x.dtype),
        scratch_shapes=[
            pltpu.VMEM((S, D), _BF),
            pltpu.VMEM((D, 3 * D), _BF),
            pltpu.VMEM((D, D), _BF),
            pltpu.VMEM((F, D), _BF),
            pltpu.VMEM((F, D), _BF),
            pltpu.VMEM((F, D), _BF),
            pltpu.VMEM((S, D), _BF),
            pltpu.VMEM((2 * D, D), _BF),
            pltpu.VMEM((_R3, D), _BF),
            pltpu.VMEM((D // 128, S // 2, 128), _F32),
            pltpu.VMEM((D // 128, -(-koff // 32) * 32, 128), _F32),
            pltpu.VMEM((_H, _DH // 2, S), _F32),
            pltpu.VMEM((_H, _DH // 2, S), _F32),
            pltpu.VMEM((_H, _DH, S), _F32),
            pltpu.VMEM((_H, _DH, S), _F32),
            pltpu.VMEM((_H, 8, S), _F32),
            pltpu.SMEM((_NZ,), jnp.int32),
            pltpu.VMEM((2, brows, _TQ), _F32),
            pltpu.VMEM((2, brows, _TQ), _F32),
            pltpu.SemaphoreType.DMA((6,)),
        ],
        compiler_params=pltpu.CompilerParams(vmem_limit_bytes=100 * 1024 * 1024),
        name="fused_block",
    )(A_x.reshape(S, D), A_wqkv, A_wo, B_w_gate.T, B_w_up.T, B_w_down)
    return out.reshape(B, S, D)
```

```python
import functools
import math

import jax
import jax.numpy as jnp
from jax import lax
import jax.experimental.pallas as pl
import jax.experimental.pallas.tpu as pltpu

_BF = jnp.bfloat16
_F32 = jnp.float32

_H = 32
_DH = 16
_EPS = 1e-5
_TQ = 512
_TK = 256
_RB = 16
_CB = 256
_R1 = 512
_R3 = 256
_NSUB = 2

_L_LO = 2.0 ** -40
_L_HI = 2.0 ** 60
_V_HI = 2.0 ** 50

_VPU_ROWS = "22222323222323232232232332323232"
_WIN = 4
_SWITCH = 16
_KP = 32
_RP = 32
_PV_SLOTS = 2.0
_P_LOAD0 = 4


def _layernorm(x):
    m = jnp.mean(x, axis=-1, keepdims=True)
    xc = x - m
    v = jnp.mean(xc * xc, axis=-1, keepdims=True)
    return xc * lax.rsqrt(v + _EPS)


def _gelu_tanh(x):
    c = math.sqrt(2.0 / math.pi)
    return 0.5 * x * (1.0 + jnp.tanh(c * (x + 0.044715 * (x * x * x))))


def _recip(x):
    r = pl.reciprocal(x, approx=True)
    return r * (2.0 - x * r)


def _pack(x):
    return pltpu.bitcast(x.astype(_BF), _F32)


def _unpack(x):
    return pltpu.bitcast(x, _BF)


def _dot(a, b):
    return lax.dot_general(a, b, (((1,), (0,)), ((), ())), preferred_element_type=_F32)


def _dot_nt(a, b):
    return lax.dot_general(a, b, (((1,), (1,)), ((), ())), preferred_element_type=_F32)


def _dot_tn(a, b):
    return lax.dot_general(a, b, (((0,), (0,)), ((), ())), preferred_element_type=_F32)


def _vpu_rows(S):
    nc = S // _TK
    nq = S // _TQ
    rl = [[16 * int(_VPU_ROWS[qb * nc + kc]) for kc in range(nc)] for qb in range(nq)]
    rmax = [max(rl[qb][kc] for qb in range(nq)) for kc in range(nc)]
    rmin = [min(rl[qb][kc] for qb in range(nq)) for kc in range(nc)]
    return rl, rmax, rmin


def _make_plan(S):
    nc = S // _TK
    nper = (S // _TQ) * nc
    rl, rmax, rmin = _vpu_rows(S)
    rv = [rl[i // nc][i % nc] for i in range(nper)]
    npcs = [(_TK - r) // 16 for r in rv]
    starts = [sum(n + _PV_SLOTS for n in npcs[:i]) + _PV_SLOTS for i in range(nper)]
    ends = [starts[i] + npcs[i] for i in range(nper)]

    def place(pos):
        i = min(t for t in range(nper) if pos <= ends[t] + 1e-6)
        return i, max(0, int(math.floor(pos - starts[i] + 1e-6)))

    tasks = [(i, r0, c0) for i in range(nper)
             for r0 in range(0, rv[i], _RB) for c0 in range(0, _TQ, _CB)]
    sched = {}
    for j, (i, r0, c0) in enumerate(tasks):
        w0 = (i // _WIN) * _WIN
        peers = [t for t in range(len(tasks)) if tasks[t][0] // _WIN == i // _WIN]
        beg = starts[w0] - _PV_SLOTS
        pos = beg + (j + 1 - peers[0]) * (ends[w0 + _WIN - 1] - beg) / len(peers)
        pos = min(max(pos, starts[i - 1] if i > 0 else 0.0), ends[i])
        sched.setdefault(place(pos), []).append(("score", i, r0, c0))
    bcast = [("bcast", d, r0) for d in range(_DH) for r0 in range(0, sum(rmax), _KP)]
    roll = [("roll", kc, r0) for kc in range(nc) for r0 in range(0, (_TK - rmin[kc]) // 2, _RP)]
    for lst in (bcast, roll):
        for j, e in enumerate(lst):
            pos = starts[0] + (j + 0.5) * (ends[_SWITCH - 1] - starts[0]) / len(lst)
            sched.setdefault(place(pos), []).append(e)
    return rv, npcs, sched


def _kernel(x_hbm, wqkv_hbm, wo_hbm, wgt_hbm, wut_hbm, wd_hbm, out_hbm,
            x_s, wqkv_s, wo_s, wgt_s, wut_s, wd_s, out_s, wqvt_s, o_s,
            k_s, kf_s, vt_s, qt_s, qf_s, acc_s, l_s, z_s, b0, b1, b2, sems,
            *, S, D):
    nq = S // _TQ
    nc = S // _TK
    ng = D // 128
    nb1 = S // _R1
    nper = nq * nc
    _, rmax, rmin = _vpu_rows(S)
    roff = [sum(rmax[:i]) for i in range(nc)]
    koff = sum(rmax)
    half = _TK // 2
    lrow = 4 * half
    rrow = lrow + 24
    krow = rrow + S // 8
    bufs = (b0, b1)
    qscale = (_DH ** -0.5) * math.log2(math.e)

    def x_copy(b, sem):
        rows = pl.ds(b * _R1, _R1)
        return pltpu.make_async_copy(x_hbm.at[rows, :], x_s.at[rows, :], sems.at[sem])

    def w_copy(c, sem):
        cols = pl.ds(c * D, D)
        return pltpu.make_async_copy(wqkv_hbm.at[:, cols], wqkv_s.at[:, cols], sems.at[sem])

    def group2():
        return [x_copy(1, 2), w_copy(0, 2)]

    def group3():
        return [x_copy(b, 3) for b in range(2, nb1)] + [w_copy(2, 3)]

    def late_copies():
        return [pltpu.make_async_copy(src, dst, sems.at[4])
                for src, dst in ((wo_hbm, wo_s), (wgt_hbm, wgt_s), (wut_hbm, wut_s), (wd_hbm, wd_s))]

    def ln_block(rb):
        return _layernorm(x_s[rb * _R1:(rb + 1) * _R1, :].astype(_F32)).astype(_BF)

    def k_block(rb, xn, split=1):
        nr = _R1 // split
        for r in range(0, _R1, nr):
            r0 = rb * _R1 + r
            k = _dot(xn[r:r + nr], wqkv_s[:, D:2 * D])
            for g in range(ng):
                lanes = slice(g * 128, (g + 1) * 128)
                k_s[g, r0 // 2:(r0 + nr) // 2, :] = _pack(k[:, lanes])
                for c in range(nc):
                    end = (c + 1) * _TK
                    if r0 < end <= r0 + nr:
                        kf_s[g, roff[c]:roff[c] + rmax[c], :] = k[end - r0 - rmax[c]:end - r0, lanes]

    def q_block(rb, xn):
        rows = slice(rb * _R1, (rb + 1) * _R1)
        qt = _dot_nt(wqvt_s[0:D, :], xn) * qscale
        for h in range(_H):
            qh = qt[h * _DH:(h + 1) * _DH]
            qt_s.at[h][:, rows] = _pack(qh)
            qf_s[h, :, rows] = qh

    def v_block(rb, xn):
        rows = slice(rb * _R1, (rb + 1) * _R1)
        vt = _dot_nt(wqvt_s[D:2 * D, :], xn)
        for h in range(_H):
            vt_s.at[h][:, rows] = _pack(vt[h * _DH:(h + 1) * _DH])
        return jnp.max(jnp.abs(vt).reshape(D // 8, 8, _R1), axis=0)

    def head_lanes(h):
        lane0 = (h & 7) * _DH
        return h >> 3, lane0, (128 - lane0) & 127

    def bcast_piece(hl, u, d, r0, nr):
        idx = jnp.full((nr, 128), hl[1] + d, jnp.int32)
        row = krow + (d // 4) * koff + r0
        col = (d % 4) * 128
        bufs[u][0, row:row + nr, col:col + 128] = jnp.take_along_axis(
            kf_s[hl[0], r0:r0 + nr, :], idx, axis=1)

    def k_slot(kc, r0):
        return rrow + (kc // 4) * half + r0, (kc % 4) * 128

    def rolled_keys(hl, rows):
        return pltpu.roll(k_s[hl[0], rows, :], hl[2], 1)

    def roll_piece(hl, u, kc, r0, nr):
        row, col = k_slot(kc, r0)
        bufs[u][0, row:row + nr, col:col + 128] = rolled_keys(
            hl, slice(kc * half + r0, kc * half + r0 + nr))

    x_copy(0, 0).start()
    w_copy(1, 1).start()
    for i in range(3):
        z_s[i] = 0
    b2[0, 2 * half:4 * half, :] = jnp.zeros((2 * half, _TQ), _F32)
    x_copy(0, 0).wait()
    for cp in group2():
        cp.start()
    xns = [ln_block(0)]
    w_copy(1, 1).wait()
    k_block(0, xns[0])
    for cp in group2():
        cp.wait()
    for cp in group3():
        cp.start()
    xns.append(ln_block(1))
    k_block(1, xns[1], 4)
    wqvt_s[0:D, :] = wqkv_s[:, 0:D].T
    q_block(0, xns[0])
    for cp in group3():
        cp.wait()
    for cp in late_copies():
        cp.start()
    q_block(1, xns[1])
    for rb in range(2, nb1):
        xns.append(ln_block(rb))
        k_block(rb, xns[rb])
    wqvt_s[D:2 * D, :] = wqkv_s[:, 2 * D:3 * D].T
    for d in range(_DH):
        bcast_piece(head_lanes(0), 0, d, 0, koff)
    for kc in range(nc):
        roll_piece(head_lanes(0), 0, kc, 0, half)
    vmax = None
    for rb, xn in enumerate(xns):
        if rb > 1:
            q_block(rb, xn)
        vm = v_block(rb, xn)
        vmax = vm if vmax is None else jnp.maximum(vmax, vm)
    for cp in late_copies():
        cp.wait()

    def p_group(buf, slot, g):
        cols = slice((g // 8) * 256, (g // 8 + 1) * 256)
        sub = 7 - g % 8
        return [buf[0, slot * half + (kt * 8 + sub) * 8:slot * half + (kt * 8 + sub + 1) * 8, cols]
                for kt in range(2)]

    def pv_dot(h, kc, groups):
        sets = []
        for st in range(2):
            rows = [groups[st * 8 + 7 - sub][kt] for kt in range(2) for sub in range(8)]
            sets.append(jnp.concatenate(rows, axis=0))
        pm = jnp.concatenate(sets, axis=1)
        return _dot(_unpack(vt_s[h, :, kc * _TK:(kc + 1) * _TK]), _unpack(pm))

    rvs, npcs, sched = _make_plan(S)

    def stage(u, i):
        return b2 if i >= _SWITCH else bufs[1 - u]

    def pair_body(hh, acc):
        cnt = [0]
        z0 = z_s[0]
        z1 = z_s[1]
        z2 = z_s[2]

        def score_task(u, h, i, r0, c0, lsum, tail):
            qb, kc = divmod(i, nc)
            dst = stage(u, i).at[z2]
            z = z0 * (cnt[0] + 2)
            cnt[0] += 1
            qv = qf_s.at[h + z]
            kv = bufs[u].at[z]
            accs = [None] * (_CB // 128)
            for d in range(_DH):
                row = krow + (d // 4) * koff + roff[kc] + rmax[kc] - rvs[i] + r0
                kb = kv[row:row + _RB, (d % 4) * 128:(d % 4 + 1) * 128]
                for cc in range(_CB // 128):
                    col = qb * _TQ + c0 + cc * 128
                    t = kb * qv[d:d + 1, col:col + 128]
                    accs[cc] = t if accs[cc] is None else accs[cc] + t
            r = (i % 4) * _TK + _TK - rvs[i] + r0
            vrow = lrow + (qb % 2) * 8
            for cc in range(_CB // 128):
                p = jnp.exp2(accs[cc])
                ps = p[0:8] + p[8:16]
                ct = c0 // 128 + cc
                lanes = slice(ct * 128, (ct + 1) * 128)
                dst[r // 2:(r + _RB) // 2, lanes] = _pack(p)
                if ct in lsum:
                    ps = lsum[ct] + ps
                elif ct in tail:
                    ps = ps + jnp.minimum(tail[ct], 0.0)
                lsum[ct] = ps
                tail[ct] = ps
                dst[vrow:vrow + 8, lanes] = ps

        loaded = {}
        for u in range(2):
            h = hh * 2 + u
            hn = head_lanes(jnp.minimum(h + 1, _H - 1))
            tail = {}
            lsums = [dict() for _ in range(nq)]

            def side_work(i, pi):
                for e in sched.get((i, pi), []):
                    if e[0] == "score":
                        score_task(u, h, e[1], e[2], e[3], lsums[e[1] // nc], tail)
                    elif e[0] == "bcast":
                        bcast_piece(hn, 1 - u, e[1], e[2], min(_KP, koff - e[2]))
                    else:
                        roll_piece(hn, 1 - u, e[1], e[2],
                                   min(_RP, (_TK - rmin[e[1]]) // 2 - e[2]))

            for i in range(nper):
                qb, kc = divmod(i, nc)
                cols = slice(qb * _TQ, (qb + 1) * _TQ)
                buf = stage(u, i)
                row, col = k_slot(kc, 0)
                kk = _unpack(bufs[u][0, row:row + (_TK - rvs[i]) // 2, col:col + 128])
                s = _dot(kk[:, 0:_DH], _unpack(qt_s[h, :, cols]))

                i2 = (i - 2) % nper
                pqb, pkc = divmod(i2, nc)
                ph = h if i >= 2 else jnp.maximum(h - 1, 0)
                groups = loaded.pop((u, i2) if i >= 2 else (u - 1, i2), None)
                if groups is None:
                    groups = [p_group(stage(u, i2), i2 % 4, g) for g in range(16)]
                pv = pv_dot(ph, pkc, groups)
                acc = pv if pkc == 0 else pv + acc
                if pkc == nc - 1:
                    acc_s[ph, :, pqb * _TQ:(pqb + 1) * _TQ] = acc

                reload = i not in (0, _SWITCH) and not (u == 1 and i == nper - 1)
                groups = []
                side_work(i, 0)
                for pi in range(npcs[i]):
                    p = jnp.exp2(s[pi * 16:(pi + 1) * 16])
                    ps = p[0:8] + p[8:16]
                    l8 = ps if (kc == 0 and pi == 0) else l8 + ps
                    row = (i % 4) * half + pi * 8
                    buf.at[z1][row:row + 8, :] = _pack(p)
                    side_work(i, pi + 1)
                    if reload:
                        want = max(0, (16 * (pi + 1 - _P_LOAD0)) // (npcs[i] - _P_LOAD0))
                        while len(groups) < want:
                            groups.append(p_group(buf, (i - 1) % 4, len(groups)))
                if reload:
                    loaded[(u, i - 1)] = groups
                if kc == nc - 1:
                    buf.at[z1][lrow + 16:lrow + 24, :] = l8
                    vrow = lrow + (qb % 2) * 8
                    l_s[h, :, cols] = buf[0, lrow + 16:lrow + 24, :] + buf[0, vrow:vrow + 8, :]
        return acc

    acc = lax.fori_loop(0, _H // 2, pair_body, jnp.zeros((_DH, _TQ), _F32))
    for j in (2, 1):
        acc = pv_dot(_H - 1, nc - j, [p_group(b2, (nper - j) % 4, g) for g in range(16)]) + acc
    acc_s[_H - 1, :, S - _TQ:S] = acc

    def max_shifted_attention():
        nt = S // 128

        def tile(t, c):
            h = t // nt
            cols = pl.ds(pl.multiple_of((t % nt) * 128, 128), 128)
            kk = _unpack(rolled_keys(head_lanes(h), slice(None)))
            s = _dot(kk[:, 0:_DH], _unpack(qt_s[h, :, cols]))
            p = jnp.exp2(s - jnp.max(s, axis=0, keepdims=True))
            p = p * (1.0 / jnp.sum(p, axis=0, keepdims=True))
            acc_s[h, :, cols] = _dot(_unpack(vt_s[h]), p.astype(_BF))
            l_s[h, :, cols] = jnp.full((8, 128), 0.125, _F32)
            return c
        lax.fori_loop(0, _H * nt, tile, 0)

    rblk = _R3 * _NSUB
    nblk = S // rblk

    def attn_rows(rows):
        l = jnp.sum(l_s[:, :, rows], axis=1, keepdims=True)
        ot = (acc_s[:, :, rows] * _recip(l)).reshape(D, _R3).astype(_BF)
        ok = jnp.logical_and(l >= _L_LO, l <= _L_HI)
        return ot.T, jnp.sum(jnp.where(ok, 0.0, 1.0), axis=0)

    def ffn_body(t, bad):
        subs = [pl.ds(pl.multiple_of(t * rblk + i * _R3, _R3), _R3) for i in range(_NSUB)]
        h1 = []
        for i, rows in enumerate(subs):
            if i == 0:
                o = o_s[...]
            else:
                o, b = attn_rows(rows)
                bad = bad + b
            h1.append(_dot(o, wo_s[...]) + x_s[rows, :].astype(_F32))
        act = []
        for i in range(_NSUB):
            hn = _layernorm(h1[i]).astype(_BF)
            gate = _dot_nt(wgt_s[...], hn)
            up = _dot_nt(wut_s[...], hn)
            act.append((_gelu_tanh(gate) * up).astype(_BF))
        nxt = jnp.minimum(t + 1, nblk - 1) * rblk
        o_s[...], b = attn_rows(pl.ds(pl.multiple_of(nxt, _R3), _R3))
        bad = bad + b
        for i, rows in enumerate(subs):
            out_s[rows, :] = (_dot_tn(act[i], wd_s[...]) + h1[i]).astype(_BF)
            pltpu.make_async_copy(out_s.at[rows, :], out_hbm.at[rows, :], sems.at[5]).start()
        return bad

    o_s[...], bad0 = attn_rows(pl.ds(0, _R3))
    vmax = jnp.max(vmax, axis=0, keepdims=True)
    for c in range(0, _R1, _R3):
        bad0 = bad0 + jnp.where(vmax[:, c:c + _R3] <= _V_HI, 0.0, 1.0)

    def one_pass(state):
        p, _ = state
        bad = lax.fori_loop(0, nblk, ffn_body, bad0)
        redo = jnp.logical_and(p == 0, jnp.sum(bad) > 0.0)

        @pl.when(redo)
        def _():
            max_shifted_attention()
            o_s[...] = attn_rows(pl.ds(0, _R3))[0]

        pltpu.make_async_copy(out_s, out_hbm, sems.at[5]).wait()
        return p + 1, redo.astype(jnp.int32)

    lax.while_loop(lambda st: st[1] > 0, one_pass, (jnp.int32(0), jnp.int32(1)))


@jax.jit
def pallas_sequential_preLN__softmax_full_mha__geglu_ffn__prompt_kernel(
    A_x: jax.Array,
    A_wqkv: jax.Array,
    A_wo: jax.Array,
    B_x: jax.Array,
    B_w_gate: jax.Array,
    B_w_up: jax.Array,
    B_w_down: jax.Array,
):
    B, S, D = A_x.shape
    F = B_w_gate.shape[1]
    assert B == 1 and D == _H * _DH and len(_VPU_ROWS) == (S // _TQ) * (S // _TK)
    assert _SWITCH % (S // _TK) == 0 and _SWITCH % _WIN == 0
    koff = sum(_vpu_rows(S)[1])
    brows = 2 * _TK + 24 + S // 8 + 4 * koff
    hbm = pl.BlockSpec(memory_space=pl.ANY)
    out = pl.pallas_call(
        functools.partial(_kernel, S=S, D=D),
        in_specs=[hbm] * 6,
        out_specs=hbm,
        out_shape=jax.ShapeDtypeStruct((S, D), A_x.dtype),
        scratch_shapes=[
            pltpu.VMEM((S, D), _BF),
            pltpu.VMEM((D, 3 * D), _BF),
            pltpu.VMEM((D, D), _BF),
            pltpu.VMEM((F, D), _BF),
            pltpu.VMEM((F, D), _BF),
            pltpu.VMEM((F, D), _BF),
            pltpu.VMEM((S, D), _BF),
            pltpu.VMEM((2 * D, D), _BF),
            pltpu.VMEM((_R3, D), _BF),
            pltpu.VMEM((D // 128, S // 2, 128), _F32),
            pltpu.VMEM((D // 128, -(-koff // 32) * 32, 128), _F32),
            pltpu.VMEM((_H, _DH // 2, S), _F32),
            pltpu.VMEM((_H, _DH // 2, S), _F32),
            pltpu.VMEM((_H, _DH, S), _F32),
            pltpu.VMEM((_H, _DH, S), _F32),
            pltpu.VMEM((_H, 8, S), _F32),
            pltpu.SMEM((3,), jnp.int32),
            pltpu.VMEM((2, brows, _TQ), _F32),
            pltpu.VMEM((2, brows, _TQ), _F32),
            pltpu.VMEM((2, 2 * _TK + 24, _TQ), _F32),
            pltpu.SemaphoreType.DMA((6,)),
        ],
        compiler_params=pltpu.CompilerParams(vmem_limit_bytes=100 * 1024 * 1024),
        name="fused_block",
    )(A_x.reshape(S, D), A_wqkv, A_wo, B_w_gate.T, B_w_up.T, B_w_down)
    return out.reshape(B, S, D)
```

```python
import functools
import math

import jax
import jax.numpy as jnp
from jax import lax
import jax.experimental.pallas as pl
import jax.experimental.pallas.tpu as pltpu

_BF = jnp.bfloat16
_F32 = jnp.float32

_H = 32
_DH = 16
_EPS = 1e-5
_TQ = 512
_TK = 256
_RB = 16
_CB = 256
_R1 = 512
_R3 = 256
_NSUB = 2

_L_LO = 2.0 ** -40
_L_HI = 2.0 ** 100
_V_HI = 2.0 ** 24

_VPU_ROWS = "22222323222323232232232332323232"
_WIN = 4
_SWITCH = 16
_KP = 32
_RP = 32
_PV_SLOTS = 2.0
_P_LOAD0 = 4


def _layernorm(x):
    m = jnp.mean(x, axis=-1, keepdims=True)
    xc = x - m
    v = jnp.mean(xc * xc, axis=-1, keepdims=True)
    return xc * lax.rsqrt(v + _EPS)


def _gelu_tanh(x):
    c = math.sqrt(2.0 / math.pi)
    return 0.5 * x * (1.0 + jnp.tanh(c * (x + 0.044715 * (x * x * x))))


def _recip(x):
    r = pl.reciprocal(x, approx=True)
    return r * (2.0 - x * r)


def _pack(x):
    return pltpu.bitcast(x.astype(_BF), _F32)


def _unpack(x):
    return pltpu.bitcast(x, _BF)


def _dot(a, b):
    return lax.dot_general(a, b, (((1,), (0,)), ((), ())), preferred_element_type=_F32)


def _dot_nt(a, b):
    return lax.dot_general(a, b, (((1,), (1,)), ((), ())), preferred_element_type=_F32)


def _vpu_rows(S):
    nc = S // _TK
    nq = S // _TQ
    rl = [[16 * int(_VPU_ROWS[qb * nc + kc]) for kc in range(nc)] for qb in range(nq)]
    rmax = [max(rl[qb][kc] for qb in range(nq)) for kc in range(nc)]
    rmin = [min(rl[qb][kc] for qb in range(nq)) for kc in range(nc)]
    return rl, rmax, rmin


def _make_plan(S):
    nc = S // _TK
    nper = (S // _TQ) * nc
    rl, rmax, rmin = _vpu_rows(S)
    rv = [rl[i // nc][i % nc] for i in range(nper)]
    npcs = [(_TK - r) // 16 for r in rv]
    starts = [sum(n + _PV_SLOTS for n in npcs[:i]) + _PV_SLOTS for i in range(nper)]
    ends = [starts[i] + npcs[i] for i in range(nper)]

    def place(pos):
        i = min(t for t in range(nper) if pos <= ends[t] + 1e-6)
        return i, max(0, int(math.floor(pos - starts[i] + 1e-6)))

    tasks = [(i, r0, c0) for i in range(nper)
             for r0 in range(0, rv[i], _RB) for c0 in range(0, _TQ, _CB)]
    sched = {}
    for j, (i, r0, c0) in enumerate(tasks):
        w0 = (i // _WIN) * _WIN
        peers = [t for t in range(len(tasks)) if tasks[t][0] // _WIN == i // _WIN]
        beg = starts[w0] - _PV_SLOTS
        pos = beg + (j + 1 - peers[0]) * (ends[w0 + _WIN - 1] - beg) / len(peers)
        pos = min(max(pos, starts[i - 1] if i > 0 else 0.0), ends[i])
        sched.setdefault(place(pos), []).append(("score", i, r0, c0))
    bcast = [("bcast", d, r0) for d in range(_DH) for r0 in range(0, sum(rmax), _KP)]
    roll = [("roll", kc, r0) for kc in range(nc) for r0 in range(0, (_TK - rmin[kc]) // 2, _RP)]
    for lst in (bcast, roll):
        for j, e in enumerate(lst):
            pos = starts[0] + (j + 0.5) * (ends[_SWITCH - 1] - starts[0]) / len(lst)
            sched.setdefault(place(pos), []).append(e)
    return rv, npcs, sched


def _kernel(x_hbm, wqkv_hbm, wo_hbm, wgt_hbm, wut_hbm, wd_hbm, out_hbm,
            x_s, wqkv_s, wo_s, wgt_s, wut_s, wd_s, out_s, wqvt_s, o_s,
            k_s, kf_s, vt_s, qt_s, qf_s, acc_s, l_s, z_s, b0, b1, b2, sems,
            *, S, D):
    nq = S // _TQ
    nc = S // _TK
    ng = D // 128
    nb1 = S // _R1
    nper = nq * nc
    _, rmax, rmin = _vpu_rows(S)
    roff = [sum(rmax[:i]) for i in range(nc)]
    koff = sum(rmax)
    half = _TK // 2
    lrow = 4 * half
    rrow = lrow + 24
    krow = rrow + S // 8
    bufs = (b0, b1)
    qscale = (_DH ** -0.5) * math.log2(math.e)

    def x_copy(b, sem):
        rows = pl.ds(b * _R1, _R1)
        return pltpu.make_async_copy(x_hbm.at[rows, :], x_s.at[rows, :], sems.at[sem])

    def w_copy(c, sem):
        cols = pl.ds(c * D, D)
        return pltpu.make_async_copy(wqkv_hbm.at[:, cols], wqkv_s.at[:, cols], sems.at[sem])

    def group2():
        return [x_copy(1, 2), w_copy(0, 2)]

    def group3():
        return [x_copy(b, 3) for b in range(2, nb1)] + [w_copy(2, 3)]

    def late_copies():
        return [pltpu.make_async_copy(src, dst, sems.at[4])
                for src, dst in ((wo_hbm, wo_s), (wgt_hbm, wgt_s), (wut_hbm, wut_s), (wd_hbm, wd_s))]

    def ln_block(rb):
        return _layernorm(x_s[rb * _R1:(rb + 1) * _R1, :].astype(_F32)).astype(_BF)

    def k_block(rb, xn, split=1):
        nr = _R1 // split
        for r in range(0, _R1, nr):
            r0 = rb * _R1 + r
            k = _dot(xn[r:r + nr], wqkv_s[:, D:2 * D])
            for g in range(ng):
                lanes = slice(g * 128, (g + 1) * 128)
                k_s[g, r0 // 2:(r0 + nr) // 2, :] = _pack(k[:, lanes])
                for c in range(nc):
                    end = (c + 1) * _TK
                    if r0 < end <= r0 + nr:
                        kf_s[g, roff[c]:roff[c] + rmax[c], :] = k[end - r0 - rmax[c]:end - r0, lanes]

    def q_block(rb, xn):
        rows = slice(rb * _R1, (rb + 1) * _R1)
        qt = _dot_nt(wqvt_s[0:D, :], xn) * qscale
        for h in range(_H):
            qh = qt[h * _DH:(h + 1) * _DH]
            qt_s.at[h][:, rows] = _pack(qh)
            qf_s[h, :, rows] = qh

    def v_block(rb, xn):
        rows = slice(rb * _R1, (rb + 1) * _R1)
        vt = _dot_nt(wqvt_s[D:2 * D, :], xn)
        for h in range(_H):
            vt_s.at[h][:, rows] = _pack(vt[h * _DH:(h + 1) * _DH])
        return jnp.max(jnp.abs(vt).reshape(D // 8, 8, _R1), axis=0)

    def head_lanes(h):
        lane0 = (h & 7) * _DH
        return h >> 3, lane0, (128 - lane0) & 127

    def bcast_piece(hl, u, d, r0, nr):
        idx = jnp.full((nr, 128), hl[1] + d, jnp.int32)
        row = krow + (d // 4) * koff + r0
        col = (d % 4) * 128
        bufs[u][0, row:row + nr, col:col + 128] = jnp.take_along_axis(
            kf_s[hl[0], r0:r0 + nr, :], idx, axis=1)

    def k_slot(kc, r0):
        return rrow + (kc // 4) * half + r0, (kc % 4) * 128

    def rolled_keys(hl, rows):
        return pltpu.roll(k_s[hl[0], rows, :], hl[2], 1)

    def roll_piece(hl, u, kc, r0, nr):
        row, col = k_slot(kc, r0)
        bufs[u][0, row:row + nr, col:col + 128] = rolled_keys(
            hl, slice(kc * half + r0, kc * half + r0 + nr))

    x_copy(0, 0).start()
    w_copy(1, 1).start()
    for i in range(3):
        z_s[i] = 0
    b2[0, 2 * half:4 * half, :] = jnp.zeros((2 * half, _TQ), _F32)
    x_copy(0, 0).wait()
    for cp in group2():
        cp.start()
    xns = [ln_block(0)]
    w_copy(1, 1).wait()
    k_block(0, xns[0])
    for cp in group2():
        cp.wait()
    for cp in group3():
        cp.start()
    xns.append(ln_block(1))
    k_block(1, xns[1], 4)
    wqvt_s[0:D, :] = wqkv_s[:, 0:D].T
    q_block(0, xns[0])
    for cp in group3():
        cp.wait()
    for cp in late_copies():
        cp.start()
    q_block(1, xns[1])
    xns.append(ln_block(2))
    k_block(2, xns[2], 2)
    wqvt_s[D:2 * D, :] = wqkv_s[:, 2 * D:3 * D].T
    vmax = v_block(0, xns[0])
    xns.append(ln_block(3))
    k_block(3, xns[3], 2)
    vmax = jnp.maximum(vmax, v_block(1, xns[1]))
    for d in range(_DH):
        bcast_piece(head_lanes(0), 0, d, 0, koff)
    for kc in range(nc):
        roll_piece(head_lanes(0), 0, kc, 0, half)
    for rb in (2, 3):
        q_block(rb, xns[rb])
        vmax = jnp.maximum(vmax, v_block(rb, xns[rb]))
    for cp in late_copies():
        cp.wait()

    def p_group(buf, slot, g):
        cols = slice((g // 8) * 256, (g // 8 + 1) * 256)
        sub = 7 - g % 8
        return [buf[0, slot * half + (kt * 8 + sub) * 8:slot * half + (kt * 8 + sub + 1) * 8, cols]
                for kt in range(2)]

    def pv_dot(h, kc, groups):
        sets = []
        for st in range(2):
            rows = [groups[st * 8 + 7 - sub][kt] for kt in range(2) for sub in range(8)]
            sets.append(jnp.concatenate(rows, axis=0))
        pm = jnp.concatenate(sets, axis=1)
        return _dot(_unpack(vt_s[h, :, kc * _TK:(kc + 1) * _TK]), _unpack(pm))

    rvs, npcs, sched = _make_plan(S)

    def stage(u, i):
        return b2 if i >= _SWITCH else bufs[1 - u]

    def pair_body(hh, acc):
        cnt = [0]
        z0 = z_s[0]
        z1 = z_s[1]
        z2 = z_s[2]

        def score_task(u, h, i, r0, c0, lsum, tail):
            qb, kc = divmod(i, nc)
            dst = stage(u, i).at[z2]
            z = z0 * (cnt[0] + 2)
            cnt[0] += 1
            qv = qf_s.at[h + z]
            kv = bufs[u].at[z]
            accs = [None] * (_CB // 128)
            for d in range(_DH):
                row = krow + (d // 4) * koff + roff[kc] + rmax[kc] - rvs[i] + r0
                kb = kv[row:row + _RB, (d % 4) * 128:(d % 4 + 1) * 128]
                for cc in range(_CB // 128):
                    col = qb * _TQ + c0 + cc * 128
                    t = kb * qv[d:d + 1, col:col + 128]
                    accs[cc] = t if accs[cc] is None else accs[cc] + t
            r = (i % 4) * _TK + _TK - rvs[i] + r0
            vrow = lrow + (qb % 2) * 8
            for cc in range(_CB // 128):
                p = jnp.exp2(accs[cc])
                ps = p[0:8] + p[8:16]
                ct = c0 // 128 + cc
                lanes = slice(ct * 128, (ct + 1) * 128)
                dst[r // 2:(r + _RB) // 2, lanes] = _pack(p)
                if ct in lsum:
                    ps = lsum[ct] + ps
                elif ct in tail:
                    ps = ps + jnp.minimum(tail[ct], 0.0)
                lsum[ct] = ps
                tail[ct] = ps
                dst[vrow:vrow + 8, lanes] = ps

        loaded = {}
        for u in range(2):
            h = hh * 2 + u
            hn = head_lanes(jnp.minimum(h + 1, _H - 1))
            tail = {}
            lsums = [dict() for _ in range(nq)]

            def side_work(i, pi):
                for e in sched.get((i, pi), []):
                    if e[0] == "score":
                        score_task(u, h, e[1], e[2], e[3], lsums[e[1] // nc], tail)
                    elif e[0] == "bcast":
                        bcast_piece(hn, 1 - u, e[1], e[2], min(_KP, koff - e[2]))
                    else:
                        roll_piece(hn, 1 - u, e[1], e[2],
                                   min(_RP, (_TK - rmin[e[1]]) // 2 - e[2]))

            for i in range(nper):
                qb, kc = divmod(i, nc)
                cols = slice(qb * _TQ, (qb + 1) * _TQ)
                buf = stage(u, i)
                row, col = k_slot(kc, 0)
                kk = _unpack(bufs[u][0, row:row + (_TK - rvs[i]) // 2, col:col + 128])
                s = _dot(kk[:, 0:_DH], _unpack(qt_s[h, :, cols]))

                i2 = (i - 2) % nper
                pqb, pkc = divmod(i2, nc)
                ph = h if i >= 2 else jnp.maximum(h - 1, 0)
                groups = loaded.pop((u, i2) if i >= 2 else (u - 1, i2), None)
                if groups is None:
                    groups = [p_group(stage(u, i2), i2 % 4, g) for g in range(16)]
                pv = pv_dot(ph, pkc, groups)
                acc = pv if pkc == 0 else pv + acc
                if pkc == nc - 1:
                    acc_s[ph, :, pqb * _TQ:(pqb + 1) * _TQ] = acc

                reload = i not in (0, _SWITCH) and not (u == 1 and i == nper - 1)
                groups = []
                side_work(i, 0)
                for pi in range(npcs[i]):
                    p = jnp.exp2(s[pi * 16:(pi + 1) * 16])
                    ps = p[0:8] + p[8:16]
                    l8 = ps if (kc == 0 and pi == 0) else l8 + ps
                    row = (i % 4) * half + pi * 8
                    buf.at[z1][row:row + 8, :] = _pack(p)
                    side_work(i, pi + 1)
                    if reload:
                        want = max(0, (16 * (pi + 1 - _P_LOAD0)) // (npcs[i] - _P_LOAD0))
                        while len(groups) < want:
                            groups.append(p_group(buf, (i - 1) % 4, len(groups)))
                if reload:
                    loaded[(u, i - 1)] = groups
                if kc == nc - 1:
                    buf.at[z1][lrow + 16:lrow + 24, :] = l8
                    vrow = lrow + (qb % 2) * 8
                    l_s[h, :, cols] = buf[0, lrow + 16:lrow + 24, :] + buf[0, vrow:vrow + 8, :]
        return acc

    acc = lax.fori_loop(0, _H // 2, pair_body, jnp.zeros((_DH, _TQ), _F32))
    for j in (2, 1):
        acc = pv_dot(_H - 1, nc - j, [p_group(b2, (nper - j) % 4, g) for g in range(16)]) + acc
    acc_s[_H - 1, :, S - _TQ:S] = acc

    def max_shifted_attention():
        nt = S // 128

        def tile(t, c):
            h = t // nt
            cols = pl.ds(pl.multiple_of((t % nt) * 128, 128), 128)
            kk = _unpack(rolled_keys(head_lanes(h), slice(None)))
            s = _dot(kk[:, 0:_DH], _unpack(qt_s[h, :, cols]))
            p = jnp.exp2(s - jnp.max(s, axis=0, keepdims=True))
            p = p * (1.0 / jnp.sum(p, axis=0, keepdims=True))
            acc_s[h, :, cols] = _dot(_unpack(vt_s[h]), p.astype(_BF))
            l_s[h, :, cols] = jnp.full((8, 128), 0.125, _F32)
            return c
        lax.fori_loop(0, _H * nt, tile, 0)

    rblk = _R3 * _NSUB
    nblk = S // rblk

    def attn_rows(rows):
        l = jnp.sum(l_s[:, :, rows], axis=1, keepdims=True)
        ot = (acc_s[:, :, rows] * _recip(l)).reshape(D, _R3).astype(_BF)
        ok = jnp.logical_and(l >= _L_LO, l <= _L_HI)
        return ot.T, jnp.sum(jnp.where(ok, 0.0, 1.0), axis=0)

    def ffn_body(t, bad):
        subs = [pl.ds(pl.multiple_of(t * rblk + i * _R3, _R3), _R3) for i in range(_NSUB)]
        h1 = []
        for i, rows in enumerate(subs):
            if i == 0:
                o = o_s[...]
            else:
                o, b = attn_rows(rows)
                bad = bad + b
            h1.append(_dot(o, wo_s[...]) + x_s[rows, :].astype(_F32))
        act = []
        for i in range(_NSUB):
            hn = _layernorm(h1[i]).astype(_BF)
            gate = _dot_nt(wgt_s[...], hn)
            up = _dot_nt(wut_s[...], hn)
            act.append((_gelu_tanh(gate) * up).astype(_BF))
        nxt = jnp.minimum(t + 1, nblk - 1) * rblk
        o_s[...], b = attn_rows(pl.ds(pl.multiple_of(nxt, _R3), _R3))
        bad = bad + b
        for i, rows in enumerate(subs):
            cw = 128 if i == _NSUB - 1 else D
            a = act[i].T
            for c0 in range(0, D, cw):
                cols = pl.ds(c0, cw)
                out_s[rows, cols] = (_dot(a, wd_s[:, cols]) + h1[i][:, c0:c0 + cw]).astype(_BF)
                pltpu.make_async_copy(out_s.at[rows, cols], out_hbm.at[rows, cols],
                                      sems.at[5]).start()
        return bad

    o_s[...], bad0 = attn_rows(pl.ds(0, _R3))
    vmax = jnp.max(vmax, axis=0, keepdims=True)
    for c in range(0, _R1, _R3):
        bad0 = bad0 + jnp.where(vmax[:, c:c + _R3] <= _V_HI, 0.0, 1.0)

    def one_pass(state):
        p, _ = state
        bad = lax.fori_loop(0, nblk, ffn_body, bad0)
        redo = jnp.logical_and(p == 0, jnp.sum(bad) > 0.0)

        @pl.when(redo)
        def _():
            max_shifted_attention()
            o_s[...] = attn_rows(pl.ds(0, _R3))[0]

        pltpu.make_async_copy(out_s, out_hbm, sems.at[5]).wait()
        return p + 1, redo.astype(jnp.int32)

    lax.while_loop(lambda st: st[1] > 0, one_pass, (jnp.int32(0), jnp.int32(1)))


@jax.jit
def pallas_sequential_preLN__softmax_full_mha__geglu_ffn__prompt_kernel(
    A_x: jax.Array,
    A_wqkv: jax.Array,
    A_wo: jax.Array,
    B_x: jax.Array,
    B_w_gate: jax.Array,
    B_w_up: jax.Array,
    B_w_down: jax.Array,
):
    B, S, D = A_x.shape
    F = B_w_gate.shape[1]
    assert B == 1 and D == _H * _DH and len(_VPU_ROWS) == (S // _TQ) * (S // _TK)
    assert S == 4 * _R1 and _SWITCH % (S // _TK) == 0 and _SWITCH % _WIN == 0
    koff = sum(_vpu_rows(S)[1])
    brows = 2 * _TK + 24 + S // 8 + 4 * koff
    hbm = pl.BlockSpec(memory_space=pl.ANY)
    out = pl.pallas_call(
        functools.partial(_kernel, S=S, D=D),
        in_specs=[hbm] * 6,
        out_specs=hbm,
        out_shape=jax.ShapeDtypeStruct((S, D), A_x.dtype),
        scratch_shapes=[
            pltpu.VMEM((S, D), _BF),
            pltpu.VMEM((D, 3 * D), _BF),
            pltpu.VMEM((D, D), _BF),
            pltpu.VMEM((F, D), _BF),
            pltpu.VMEM((F, D), _BF),
            pltpu.VMEM((F, D), _BF),
            pltpu.VMEM((S, D), _BF),
            pltpu.VMEM((2 * D, D), _BF),
            pltpu.VMEM((_R3, D), _BF),
            pltpu.VMEM((D // 128, S // 2, 128), _F32),
            pltpu.VMEM((D // 128, -(-koff // 32) * 32, 128), _F32),
            pltpu.VMEM((_H, _DH // 2, S), _F32),
            pltpu.VMEM((_H, _DH // 2, S), _F32),
            pltpu.VMEM((_H, _DH, S), _F32),
            pltpu.VMEM((_H, _DH, S), _F32),
            pltpu.VMEM((_H, 8, S), _F32),
            pltpu.SMEM((3,), jnp.int32),
            pltpu.VMEM((2, brows, _TQ), _F32),
            pltpu.VMEM((2, brows, _TQ), _F32),
            pltpu.VMEM((2, 2 * _TK + 24, _TQ), _F32),
            pltpu.SemaphoreType.DMA((6,)),
        ],
        compiler_params=pltpu.CompilerParams(vmem_limit_bytes=100 * 1024 * 1024),
        name="fused_block",
    )(A_x.reshape(S, D), A_wqkv, A_wo, B_w_gate.T, B_w_up.T, B_w_down)
    return out.reshape(B, S, D)
```

```python
import functools
import math

import jax
import jax.numpy as jnp
from jax import lax
import jax.experimental.pallas as pl
import jax.experimental.pallas.tpu as pltpu

_BF = jnp.bfloat16
_F32 = jnp.float32

_H = 32
_DH = 16
_EPS = 1e-5
_TQ = 512
_TK = 256
_RB = 16
_CB = 256
_R1 = 512
_R3 = 256
_NSUB = 2
_PRE = 16

_L_LO = 2.0 ** -40
_L_HI = 2.0 ** 100
_V_HI = 2.0 ** 24

_VPU_ROWS = "22222323222323232232232332323232"
_WIN = 4
_SWITCH = 16
_KP = 32
_RP = 32
_PV_SLOTS = 2.0
_P_LOAD0 = 4


def _layernorm(x):
    m = jnp.mean(x, axis=-1, keepdims=True)
    xc = x - m
    v = jnp.mean(xc * xc, axis=-1, keepdims=True)
    return xc * lax.rsqrt(v + _EPS)


def _gelu_tanh(x):
    c = math.sqrt(2.0 / math.pi)
    return 0.5 * x * (1.0 + jnp.tanh(c * (x + 0.044715 * (x * x * x))))


def _recip(x):
    r = pl.reciprocal(x, approx=True)
    return r * (2.0 - x * r)


def _pack(x):
    return pltpu.bitcast(x.astype(_BF), _F32)


def _unpack(x):
    return pltpu.bitcast(x, _BF)


def _dot(a, b):
    return lax.dot_general(a, b, (((1,), (0,)), ((), ())), preferred_element_type=_F32)


def _dot_nt(a, b):
    return lax.dot_general(a, b, (((1,), (1,)), ((), ())), preferred_element_type=_F32)


def _vpu_rows(S):
    nc = S // _TK
    nq = S // _TQ
    rl = [[16 * int(_VPU_ROWS[qb * nc + kc]) for kc in range(nc)] for qb in range(nq)]
    rmax = [max(rl[qb][kc] for qb in range(nq)) for kc in range(nc)]
    rmin = [min(rl[qb][kc] for qb in range(nq)) for kc in range(nc)]
    return rl, rmax, rmin


def _make_plan(S):
    nc = S // _TK
    nper = (S // _TQ) * nc
    rl, rmax, rmin = _vpu_rows(S)
    rv = [rl[i // nc][i % nc] for i in range(nper)]
    npcs = [(_TK - r) // 16 for r in rv]
    starts = [sum(n + _PV_SLOTS for n in npcs[:i]) + _PV_SLOTS for i in range(nper)]
    ends = [starts[i] + npcs[i] for i in range(nper)]

    def place(pos):
        i = min(t for t in range(nper) if pos <= ends[t] + 1e-6)
        return i, max(0, int(math.floor(pos - starts[i] + 1e-6)))

    tasks = [(i, r0, c0) for i in range(nper)
             for r0 in range(0, rv[i], _RB) for c0 in range(0, _TQ, _CB)]
    sched = {}
    for j, (i, r0, c0) in enumerate(tasks):
        w0 = (i // _WIN) * _WIN
        peers = [t for t in range(len(tasks)) if tasks[t][0] // _WIN == i // _WIN]
        beg = starts[w0] - _PV_SLOTS
        pos = beg + (j + 1 - peers[0]) * (ends[w0 + _WIN - 1] - beg) / len(peers)
        pos = min(max(pos, starts[i - 1] if i > 0 else 0.0), ends[i])
        sched.setdefault(place(pos), []).append(("score", i, r0, c0))
    bcast = [("bcast", d, r0) for d in range(_DH) for r0 in range(0, sum(rmax), _KP)]
    roll = [("roll", kc, r0) for kc in range(nc) for r0 in range(0, (_TK - rmin[kc]) // 2, _RP)]
    for lst in (bcast, roll):
        for j, e in enumerate(lst):
            pos = starts[0] + (j + 0.5) * (ends[_SWITCH - 1] - starts[0]) / len(lst)
            sched.setdefault(place(pos), []).append(e)
    return rv, npcs, sched


def _kernel(x_hbm, wqkv_hbm, wo_hbm, wgt_hbm, wut_hbm, wd_hbm, out_hbm,
            x_s, wqkv_s, wo_s, wgt_s, wut_s, wd_s, out_s, wqvt_s, o_s,
            k_s, kf_s, vt_s, qt_s, qf_s, acc_s, l_s, z_s, b0, b1, b2, sems,
            *, S, D):
    nq = S // _TQ
    nc = S // _TK
    ng = D // 128
    nb1 = S // _R1
    nper = nq * nc
    _, rmax, rmin = _vpu_rows(S)
    roff = [sum(rmax[:i]) for i in range(nc)]
    koff = sum(rmax)
    half = _TK // 2
    lrow = 4 * half
    rrow = lrow + 24
    krow = rrow + S // 8
    bufs = (b0, b1)
    qscale = (_DH ** -0.5) * math.log2(math.e)

    def x_copy(b, sem):
        rows = pl.ds(b * _R1, _R1)
        return pltpu.make_async_copy(x_hbm.at[rows, :], x_s.at[rows, :], sems.at[sem])

    def w_copy(c, sem):
        cols = pl.ds(c * D, D)
        return pltpu.make_async_copy(wqkv_hbm.at[:, cols], wqkv_s.at[:, cols], sems.at[sem])

    def group2():
        return [x_copy(1, 2), w_copy(0, 2)]

    def group3():
        return [x_copy(b, 3) for b in range(2, nb1)] + [w_copy(2, 3)]

    def late_copies():
        return [pltpu.make_async_copy(src, dst, sems.at[4])
                for src, dst in ((wo_hbm, wo_s), (wgt_hbm, wgt_s), (wut_hbm, wut_s), (wd_hbm, wd_s))]

    def ln_block(rb):
        return _layernorm(x_s[rb * _R1:(rb + 1) * _R1, :].astype(_F32)).astype(_BF)

    def k_block(rb, xn, split=1):
        nr = _R1 // split
        for r in range(0, _R1, nr):
            r0 = rb * _R1 + r
            k = _dot(xn[r:r + nr], wqkv_s[:, D:2 * D])
            for g in range(ng):
                lanes = slice(g * 128, (g + 1) * 128)
                k_s[g, r0 // 2:(r0 + nr) // 2, :] = _pack(k[:, lanes])
                for c in range(nc):
                    end = (c + 1) * _TK
                    if r0 < end <= r0 + nr:
                        kf_s[g, roff[c]:roff[c] + rmax[c], :] = k[end - r0 - rmax[c]:end - r0, lanes]

    def q_block(rb, xn):
        rows = slice(rb * _R1, (rb + 1) * _R1)
        qt = _dot_nt(wqvt_s[0:D, :], xn) * qscale
        for h in range(_H):
            qh = qt[h * _DH:(h + 1) * _DH]
            qt_s.at[h][:, rows] = _pack(qh)
            qf_s[h, :, rows] = qh

    def v_block(rb, xn):
        rows = slice(rb * _R1, (rb + 1) * _R1)
        vt = _dot_nt(wqvt_s[D:2 * D, :], xn)
        for h in range(_H):
            vt_s.at[h][:, rows] = _pack(vt[h * _DH:(h + 1) * _DH])
        return jnp.max(jnp.abs(vt).reshape(D // 8, 8, _R1), axis=0)

    def head_lanes(h):
        lane0 = (h & 7) * _DH
        return h >> 3, lane0, (128 - lane0) & 127

    def bcast_piece(hl, u, d, r0, nr):
        idx = jnp.full((nr, 128), hl[1] + d, jnp.int32)
        row = krow + (d // 4) * koff + r0
        col = (d % 4) * 128
        bufs[u][0, row:row + nr, col:col + 128] = jnp.take_along_axis(
            kf_s[hl[0], r0:r0 + nr, :], idx, axis=1)

    def k_slot(kc, r0):
        return rrow + (kc // 4) * half + r0, (kc % 4) * 128

    def rolled_keys(hl, rows):
        return pltpu.roll(k_s[hl[0], rows, :], hl[2], 1)

    def roll_piece(hl, u, kc, r0, nr):
        row, col = k_slot(kc, r0)
        bufs[u][0, row:row + nr, col:col + 128] = rolled_keys(
            hl, slice(kc * half + r0, kc * half + r0 + nr))

    x_copy(0, 0).start()
    w_copy(1, 1).start()
    for i in range(3):
        z_s[i] = 0
    b2[0, 2 * half:4 * half, :] = jnp.zeros((2 * half, _TQ), _F32)
    x_copy(0, 0).wait()
    for cp in group2():
        cp.start()
    xns = [ln_block(0)]
    w_copy(1, 1).wait()
    k_block(0, xns[0])
    for cp in group2():
        cp.wait()
    for cp in group3():
        cp.start()
    for c in range(0, D, 128):
        wqvt_s[c:c + 128, :] = wqkv_s[:, c:c + 128].T
    q_block(0, xns[0])
    xns.append(ln_block(1))
    k_block(1, xns[1], 2)
    for cp in group3():
        cp.wait()
    for cp in late_copies():
        cp.start()
    q_block(1, xns[1])
    xns.append(ln_block(2))
    k_block(2, xns[2], 2)
    wqvt_s[D:2 * D, :] = wqkv_s[:, 2 * D:3 * D].T
    vmax = v_block(0, xns[0])
    xns.append(ln_block(3))
    k_block(3, xns[3], 2)
    vmax = jnp.maximum(vmax, v_block(1, xns[1]))
    for d in range(_DH):
        bcast_piece(head_lanes(0), 0, d, 0, koff)
    for kc in range(nc):
        roll_piece(head_lanes(0), 0, kc, 0, half)
    for rb in (2, 3):
        q_block(rb, xns[rb])
        vmax = jnp.maximum(vmax, v_block(rb, xns[rb]))
    for cp in late_copies():
        cp.wait()

    def p_group(buf, slot, g):
        cols = slice((g // 8) * 256, (g // 8 + 1) * 256)
        sub = 7 - g % 8
        return [buf[0, slot * half + (kt * 8 + sub) * 8:slot * half + (kt * 8 + sub + 1) * 8, cols]
                for kt in range(2)]

    def pv_dot(h, kc, groups):
        sets = []
        for st in range(2):
            rows = [groups[st * 8 + 7 - sub][kt] for kt in range(2) for sub in range(8)]
            sets.append(jnp.concatenate(rows, axis=0))
        pm = jnp.concatenate(sets, axis=1)
        return _dot(_unpack(vt_s[h, :, kc * _TK:(kc + 1) * _TK]), _unpack(pm))

    rvs, npcs, sched = _make_plan(S)

    def stage(u, i):
        return b2 if i >= _SWITCH else bufs[1 - u]

    def pair_body(hh, acc):
        cnt = [0]
        z0 = z_s[0]
        z1 = z_s[1]
        z2 = z_s[2]

        def score_task(u, h, i, r0, c0, lsum, tail):
            qb, kc = divmod(i, nc)
            dst = stage(u, i).at[z2]
            z = z0 * (cnt[0] + 2)
            cnt[0] += 1
            qv = qf_s.at[h + z]
            kv = bufs[u].at[z]
            accs = [None] * (_CB // 128)
            for d in range(_DH):
                row = krow + (d // 4) * koff + roff[kc] + rmax[kc] - rvs[i] + r0
                kb = kv[row:row + _RB, (d % 4) * 128:(d % 4 + 1) * 128]
                for cc in range(_CB // 128):
                    col = qb * _TQ + c0 + cc * 128
                    t = kb * qv[d:d + 1, col:col + 128]
                    accs[cc] = t if accs[cc] is None else accs[cc] + t
            r = (i % 4) * _TK + _TK - rvs[i] + r0
            vrow = lrow + (qb % 2) * 8
            for cc in range(_CB // 128):
                p = jnp.exp2(accs[cc])
                ps = p[0:8] + p[8:16]
                ct = c0 // 128 + cc
                lanes = slice(ct * 128, (ct + 1) * 128)
                dst[r // 2:(r + _RB) // 2, lanes] = _pack(p)
                if ct in lsum:
                    ps = lsum[ct] + ps
                elif ct in tail:
                    ps = ps + jnp.minimum(tail[ct], 0.0)
                lsum[ct] = ps
                tail[ct] = ps
                dst[vrow:vrow + 8, lanes] = ps

        loaded = {}
        for u in range(2):
            h = hh * 2 + u
            hn = head_lanes(jnp.minimum(h + 1, _H - 1))
            tail = {}
            lsums = [dict() for _ in range(nq)]

            def side_work(i, pi):
                for e in sched.get((i, pi), []):
                    if e[0] == "score":
                        score_task(u, h, e[1], e[2], e[3], lsums[e[1] // nc], tail)
                    elif e[0] == "bcast":
                        bcast_piece(hn, 1 - u, e[1], e[2], min(_KP, koff - e[2]))
                    else:
                        roll_piece(hn, 1 - u, e[1], e[2],
                                   min(_RP, (_TK - rmin[e[1]]) // 2 - e[2]))

            for i in range(nper):
                qb, kc = divmod(i, nc)
                cols = slice(qb * _TQ, (qb + 1) * _TQ)
                buf = stage(u, i)
                row, col = k_slot(kc, 0)
                kk = _unpack(bufs[u][0, row:row + (_TK - rvs[i]) // 2, col:col + 128])
                s = _dot(kk[:, 0:_DH], _unpack(qt_s[h, :, cols]))

                i2 = (i - 2) % nper
                pqb, pkc = divmod(i2, nc)
                ph = h if i >= 2 else jnp.maximum(h - 1, 0)
                groups = loaded.pop((u, i2) if i >= 2 else (u - 1, i2), None)
                if groups is None:
                    groups = [p_group(stage(u, i2), i2 % 4, g) for g in range(16)]
                pv = pv_dot(ph, pkc, groups)
                acc = pv if pkc == 0 else pv + acc
                if pkc == nc - 1:
                    acc_s[ph, :, pqb * _TQ:(pqb + 1) * _TQ] = acc

                reload = i not in (0, _SWITCH) and not (u == 1 and i == nper - 1)
                groups = []
                side_work(i, 0)
                for pi in range(npcs[i]):
                    p = jnp.exp2(s[pi * 16:(pi + 1) * 16])
                    ps = p[0:8] + p[8:16]
                    l8 = ps if (kc == 0 and pi == 0) else l8 + ps
                    row = (i % 4) * half + pi * 8
                    buf.at[z1][row:row + 8, :] = _pack(p)
                    side_work(i, pi + 1)
                    if reload:
                        want = max(0, (16 * (pi + 1 - _P_LOAD0)) // (npcs[i] - _P_LOAD0))
                        while len(groups) < want:
                            groups.append(p_group(buf, (i - 1) % 4, len(groups)))
                if reload:
                    loaded[(u, i - 1)] = groups
                if kc == nc - 1:
                    buf.at[z1][lrow + 16:lrow + 24, :] = l8
                    vrow = lrow + (qb % 2) * 8
                    l_s[h, :, cols] = buf[0, lrow + 16:lrow + 24, :] + buf[0, vrow:vrow + 8, :]
        return acc

    acc = lax.fori_loop(0, _H // 2, pair_body, jnp.zeros((_DH, _TQ), _F32))
    for j in (2, 1):
        acc = pv_dot(_H - 1, nc - j, [p_group(b2, (nper - j) % 4, g) for g in range(16)]) + acc
    acc_s[_H - 1, :, S - _TQ:S] = acc

    def max_shifted_attention():
        nt = S // 128

        def tile(t, c):
            h = t // nt
            cols = pl.ds(pl.multiple_of((t % nt) * 128, 128), 128)
            kk = _unpack(rolled_keys(head_lanes(h), slice(None)))
            s = _dot(kk[:, 0:_DH], _unpack(qt_s[h, :, cols]))
            p = jnp.exp2(s - jnp.max(s, axis=0, keepdims=True))
            p = p * (1.0 / jnp.sum(p, axis=0, keepdims=True))
            acc_s[h, :, cols] = _dot(_unpack(vt_s[h]), p.astype(_BF))
            l_s[h, :, cols] = jnp.full((8, 128), 0.125, _F32)
            return c
        lax.fori_loop(0, _H * nt, tile, 0)

    rblk = _R3 * _NSUB
    nblk = S // rblk

    def attn_rows(rows, h0=0, h1=_H):
        l = jnp.sum(l_s[h0:h1, :, rows], axis=1, keepdims=True)
        ot = (acc_s[h0:h1, :, rows] * _recip(l)).reshape((h1 - h0) * _DH, _R3).astype(_BF)
        ok = jnp.logical_and(l >= _L_LO, l <= _L_HI)
        return ot.T, jnp.sum(jnp.where(ok, 0.0, 1.0), axis=0)

    def ffn_body(t, bad):
        subs = [pl.ds(pl.multiple_of(t * rblk + i * _R3, _R3), _R3) for i in range(_NSUB)]
        h1 = []
        for i, rows in enumerate(subs):
            res = x_s[rows, :].astype(_F32)
            if i == 0:
                res = _dot(o_s[...], wo_s[0:_PRE * _DH, :]) + res
                o, b = attn_rows(rows, _PRE, _H)
                h1.append(_dot(o, wo_s[_PRE * _DH:D, :]) + res)
            else:
                o, b = attn_rows(rows)
                h1.append(_dot(o, wo_s[...]) + res)
            bad = bad + b
        act = []
        for i in range(_NSUB):
            hn = _layernorm(h1[i]).astype(_BF)
            gate = _dot_nt(wgt_s[...], hn)
            up = _dot_nt(wut_s[...], hn)
            act.append((_gelu_tanh(gate) * up).astype(_BF))
        nxt = jnp.minimum(t + 1, nblk - 1) * rblk
        o_s[...], b = attn_rows(pl.ds(pl.multiple_of(nxt, _R3), _R3), 0, _PRE)
        bad = bad + b
        for i, rows in enumerate(subs):
            cw = 128 if i == _NSUB - 1 else D
            a = act[i].T
            for c0 in range(0, D, cw):
                cols = pl.ds(c0, cw)
                out_s[rows, cols] = (_dot(a, wd_s[:, cols]) + h1[i][:, c0:c0 + cw]).astype(_BF)
                pltpu.make_async_copy(out_s.at[rows, cols], out_hbm.at[rows, cols],
                                      sems.at[5]).start()
        return bad

    o_s[...], bad0 = attn_rows(pl.ds(0, _R3), 0, _PRE)
    vmax = jnp.max(vmax, axis=0, keepdims=True)
    for c in range(0, _R1, _R3):
        bad0 = bad0 + jnp.where(vmax[:, c:c + _R3] <= _V_HI, 0.0, 1.0)

    def one_pass(state):
        p, _ = state
        bad = lax.fori_loop(0, nblk, ffn_body, bad0)
        redo = jnp.logical_and(p == 0, jnp.sum(bad) > 0.0)

        @pl.when(redo)
        def _():
            max_shifted_attention()
            o_s[...] = attn_rows(pl.ds(0, _R3), 0, _PRE)[0]

        pltpu.make_async_copy(out_s, out_hbm, sems.at[5]).wait()
        return p + 1, redo.astype(jnp.int32)

    lax.while_loop(lambda st: st[1] > 0, one_pass, (jnp.int32(0), jnp.int32(1)))


@jax.jit
def pallas_sequential_preLN__softmax_full_mha__geglu_ffn__prompt_kernel(
    A_x: jax.Array,
    A_wqkv: jax.Array,
    A_wo: jax.Array,
    B_x: jax.Array,
    B_w_gate: jax.Array,
    B_w_up: jax.Array,
    B_w_down: jax.Array,
):
    B, S, D = A_x.shape
    F = B_w_gate.shape[1]
    assert B == 1 and D == _H * _DH and len(_VPU_ROWS) == (S // _TQ) * (S // _TK)
    assert S == 4 * _R1 and _SWITCH % (S // _TK) == 0 and _SWITCH % _WIN == 0
    koff = sum(_vpu_rows(S)[1])
    brows = 2 * _TK + 24 + S // 8 + 4 * koff
    hbm = pl.BlockSpec(memory_space=pl.ANY)
    out = pl.pallas_call(
        functools.partial(_kernel, S=S, D=D),
        in_specs=[hbm] * 6,
        out_specs=hbm,
        out_shape=jax.ShapeDtypeStruct((S, D), A_x.dtype),
        scratch_shapes=[
            pltpu.VMEM((S, D), _BF),
            pltpu.VMEM((D, 3 * D), _BF),
            pltpu.VMEM((D, D), _BF),
            pltpu.VMEM((F, D), _BF),
            pltpu.VMEM((F, D), _BF),
            pltpu.VMEM((F, D), _BF),
            pltpu.VMEM((S, D), _BF),
            pltpu.VMEM((2 * D, D), _BF),
            pltpu.VMEM((_R3, _PRE * _DH), _BF),
            pltpu.VMEM((D // 128, S // 2, 128), _F32),
            pltpu.VMEM((D // 128, -(-koff // 32) * 32, 128), _F32),
            pltpu.VMEM((_H, _DH // 2, S), _F32),
            pltpu.VMEM((_H, _DH // 2, S), _F32),
            pltpu.VMEM((_H, _DH, S), _F32),
            pltpu.VMEM((_H, _DH, S), _F32),
            pltpu.VMEM((_H, 8, S), _F32),
            pltpu.SMEM((3,), jnp.int32),
            pltpu.VMEM((2, brows, _TQ), _F32),
            pltpu.VMEM((2, brows, _TQ), _F32),
            pltpu.VMEM((2, 2 * _TK + 24, _TQ), _F32),
            pltpu.SemaphoreType.DMA((6,)),
        ],
        compiler_params=pltpu.CompilerParams(vmem_limit_bytes=100 * 1024 * 1024),
        name="fused_block",
    )(A_x.reshape(S, D), A_wqkv, A_wo, B_w_gate.T, B_w_up.T, B_w_down)
    return out.reshape(B, S, D)
```
